```python
import jax
import jax.numpy as jnp

def _softmax(x, axis=-1):
    return jax.nn.softmax(x, axis=axis)
def _gelu(x):
    return jax.nn.gelu(x, approximate=True)
def _silu(x):
    return jax.nn.silu(x)
def _sigmoid(x):
    return jax.nn.sigmoid(x)
def _layernorm(x, axis=-1, eps=1e-5):
    m = jnp.mean(x, axis=axis, keepdims=True)
    v = jnp.var(x, axis=axis, keepdims=True)
    return (x - m) / jnp.sqrt(v + eps)
def _scatter_add(tgt, idx, src, axis=0):
    return tgt.at[idx].add(src)
def _segment_sum(src, seg, n):
    return jax.ops.segment_sum(src, seg, n)
class _Rng:
    def __init__(self, key):
        self._k = key
    def _next(self):
        self._k, sub = jax.random.split(self._k)
        return sub
    def normal(self, shape):
        return jax.random.normal(self._next(), shape, dtype=jnp.bfloat16)
    def randint(self, lo, hi, shape):
        return jax.random.randint(self._next(), shape, lo, hi, dtype=jnp.int32)
    def uniform(self, shape, lo=0.0, hi=1.0):
        return jax.random.uniform(self._next(), shape, jnp.bfloat16, lo, hi)
    def permutation(self, n):
        return jax.random.permutation(self._next(), n)


kernel_name = 'concat_heads__gqa_block_cached__mha_block_cached__near_ridge'

def setup_inputs():
    _rng = _Rng(jax.random.key(int.from_bytes(__import__("os").urandom(4), "little")))
    _w = (lambda a: (lambda t: t.astype(jnp.bfloat16) if jnp.issubdtype(t.dtype, jnp.floating) else t)(jnp.asarray(a)))
    def _A_setup():
        B, Sq, D = 16, 160, 640
        Hq, Hkv, Sk, Dh = 32, 32, 512, 192
        assert Hq % Hkv == 0, (Hq, Hkv)
        return {
            "x": _w((lambda *s: _rng.normal(s) * 0.05)(B, Sq, D)),
            "k_cache": _w((lambda *s: _rng.normal(s) * 0.05)(B, Hkv, Sk, Dh)),
            "v_cache": _w((lambda *s: _rng.normal(s) * 0.05)(B, Hkv, Sk, Dh)),
            "wq": _w((lambda *s: _rng.normal(s) * 0.05)(D, Hq * Dh) * (D ** -0.5)),
            "wo": _w((lambda *s: _rng.normal(s) * 0.05)(Hq * Dh, D) * ((Hq * Dh) ** -0.5)),
        }
    _A_in = _A_setup()

    def _B_setup():
        B, Sq, D = 16, 160, 640
        H, Sk, Dh = 32, 512, 192
        return {
            "x": _w((lambda *s: _rng.normal(s) * 0.05)(B, Sq, D)),
            "k_cache": _w((lambda *s: _rng.normal(s) * 0.05)(B, H, Sk, Dh)),
            "v_cache": _w((lambda *s: _rng.normal(s) * 0.05)(B, H, Sk, Dh)),
            "wq": _w((lambda *s: _rng.normal(s) * 0.05)(D, H * Dh) * (D ** -0.5)),
            "wo": _w((lambda *s: _rng.normal(s) * 0.05)(H * Dh, D) * ((H * Dh) ** -0.5)),
        }
    _B_in = _B_setup()

    return {
        "A_x": _A_in["x"],
        "A_k_cache": _A_in["k_cache"],
        "A_v_cache": _A_in["v_cache"],
        "A_wq": _A_in["wq"],
        "A_wo": _A_in["wo"],
        "B_x": _B_in["x"],
        "B_k_cache": _B_in["k_cache"],
        "B_v_cache": _B_in["v_cache"],
        "B_wq": _B_in["wq"],
        "B_wo": _B_in["wo"],
    }

def reference(A_x, A_k_cache, A_v_cache, A_wq, A_wo, B_x, B_k_cache, B_v_cache, B_wq, B_wo):
    def _A_ref(x, k_cache, v_cache, wq, wo):
        B, Sq, D = x.shape
        Hq, Dh = 32, 192
        Hkv = k_cache.shape[1]
        rep = Hq // Hkv
        q = (lambda x, *d: x.transpose(*d))((x @ wq).reshape(B, Sq, Hq, Dh), 0, 2, 1, 3)
        k = jnp.repeat(k_cache, rep, axis=1)
        v = jnp.repeat(v_cache, rep, axis=1)
        scores = jnp.einsum("bhqd,bhkd->bhqk", q, k) * (Dh ** -0.5)
        p = _softmax(scores, axis=-1)
        o = jnp.einsum("bhqk,bhkd->bhqd", p, v)
        return (lambda x, *d: x.transpose(*d))(o, 0, 2, 1, 3).reshape(B, Sq, Hq * Dh) @ wo

    def _B_ref(x, k_cache, v_cache, wq, wo):
        B, Sq, D = x.shape
        H, Dh = 32, 192
        q = (lambda x, *d: x.transpose(*d))((x @ wq).reshape(B, Sq, H, Dh), 0, 2, 1, 3)
        scores = jnp.einsum("bhqd,bhkd->bhqk", q, k_cache) * (Dh ** -0.5)
        p = _softmax(scores, axis=-1)
        o = jnp.einsum("bhqk,bhkd->bhqd", p, v_cache)
        return (lambda x, *d: x.transpose(*d))(o, 0, 2, 1, 3).reshape(B, Sq, H * Dh) @ wo

    a = _A_ref(A_x, A_k_cache, A_v_cache, A_wq, A_wo)
    b = _B_ref(B_x, B_k_cache, B_v_cache, B_wq, B_wo)
    return jnp.concatenate([a, b], axis=-1)
```

```python
import jax
import jax.numpy as jnp
import numpy as np
import jax.experimental.pallas as pl
import jax.experimental.pallas.tpu as pltpu

_NT = (((1,), (1,)), ((), ()))


@jax.jit
def pallas_concat_heads__gqa_block_cached__mha_block_cached__near_ridge_kernel(
    A_x: jax.Array,
    A_k_cache: jax.Array,
    A_v_cache: jax.Array,
    A_wq: jax.Array,
    A_wo: jax.Array,
    B_x: jax.Array,
    B_k_cache: jax.Array,
    B_v_cache: jax.Array,
    B_wq: jax.Array,
    B_wo: jax.Array,
):
    B, Sq, D = A_x.shape
    _, H, Sk, Dh = A_k_cache.shape
    G, BB, LAG = 4, 2, 2
    NG = H // G
    c = float(Dh**-0.5 * np.log2(np.e))

    def kernel(ax, akt, avt, awq, awo, bx, bkt, bvt, bwq, bwo, out_ref, acc_ref):
        g = pl.program_id(0)
        b = pl.program_id(1)

        @pl.when(g == 0)
        def _():
            acc_ref[b] = jnp.zeros(acc_ref.shape[1:], jnp.float32)

        brs = [(ax, akt, avt, awq, awo), (bx, bkt, bvt, bwq, bwo)]
        qs = []
        for x_ref, _, _, wq, _ in brs:
            x = x_ref[...].reshape(BB * Sq, D)
            q = jnp.dot(x, wq[...], preferred_element_type=jnp.float32)
            qs.append((q * c).astype(jnp.bfloat16))
        units = [(r, bb, j) for r in range(2) for bb in range(BB) for j in range(G)]
        ps, os_ = {}, {}

        def do_s(u):
            r, bb, j = u
            qh = qs[r][bb * Sq:(bb + 1) * Sq, j * Dh:(j + 1) * Dh]
            s = jnp.dot(qh, brs[r][1][bb, j * Dh:(j + 1) * Dh, :], preferred_element_type=jnp.float32)
            m = jnp.max(s, axis=-1, keepdims=True)
            p = jnp.exp2(s - m)
            l = jnp.sum(p, axis=-1, keepdims=True)
            ps[u] = (p.astype(jnp.bfloat16), 1.0 / l)

        def do_pv(u):
            r, bb, j = u
            p, rl = ps[u]
            o = jax.lax.dot_general(p, brs[r][2][bb, j * Dh:(j + 1) * Dh, :], _NT,
                                    preferred_element_type=jnp.float32)
            os_[u] = (o * rl).astype(jnp.bfloat16)

        n = len(units)
        for i in range(n + LAG):
            if i < n:
                do_s(units[i])
            if i >= LAG:
                do_pv(units[i - LAG])
        for r in range(2):
            o = jnp.concatenate(
                [jnp.concatenate([os_[(r, bb, j)] for j in range(G)], axis=-1) for bb in range(BB)],
                axis=0)
            acc_ref[b, :, r * D:(r + 1) * D] += jnp.dot(o, brs[r][4][...], preferred_element_type=jnp.float32)

        @pl.when(g == NG - 1)
        def _():
            out_ref[...] = acc_ref[b].astype(out_ref.dtype).reshape(BB, Sq, 2 * D)

    t = lambda a: jnp.swapaxes(a, 2, 3).reshape(B, H * Dh, Sk)
    specs = [
        pl.BlockSpec((BB, Sq, D), lambda g, b: (b, 0, 0)),
        pl.BlockSpec((BB, G * Dh, Sk), lambda g, b: (b, g, 0)),
        pl.BlockSpec((BB, G * Dh, Sk), lambda g, b: (b, g, 0)),
        pl.BlockSpec((D, G * Dh), lambda g, b: (0, g)),
        pl.BlockSpec((G * Dh, D), lambda g, b: (g, 0)),
    ]
    return pl.pallas_call(
        kernel,
        grid=(NG, B // BB),
        in_specs=specs + specs,
        out_specs=pl.BlockSpec((BB, Sq, 2 * D), lambda g, b: (jnp.where(g == NG - 1, b, 0), 0, 0)),
        out_shape=jax.ShapeDtypeStruct((B, Sq, 2 * D), A_x.dtype),
        scratch_shapes=[pltpu.VMEM((B // BB, BB * Sq, 2 * D), jnp.float32)],
        compiler_params=pltpu.CompilerParams(
            dimension_semantics=("arbitrary", "arbitrary"),
            vmem_limit_bytes=100 * 1024 * 1024),
    )(A_x, t(A_k_cache), t(A_v_cache), A_wq, A_wo, B_x, t(B_k_cache), t(B_v_cache), B_wq, B_wo)
```

```python
import functools, contextlib
import jax, jax.numpy as jnp, numpy as np
from jax import lax
from jax.experimental import pallas as pl
from jax.experimental.pallas import tpu as pltpu

B,Sq,D,H,Sk,Dh = 16,160,640,32,512,192
C = float(Dh**-0.5 * np.log2(np.e))
NT = (((1,),(1,)),((),()))
f32 = jnp.float32; bf16 = jnp.bfloat16
HQ = Sq//2

def build(G=4, BB=2, vmem=110, lag=2, flags=None, NS=3, inter=0, order="sfp", prof=False, exact=True, nodma=False):
    ns = (lambda n: jax.named_scope(n)) if prof else (lambda n: contextlib.nullcontext())
    NG = H//G; NB = B//BB; T = NG*NB; M = BB*Sq; W = G*Dh
    assert NB & (NB-1) == 0
    LB = NB.bit_length()-1
    def kernel(ax, akt, avt, awq, awo, bx, bkt, bvt, bwq, bwo, out_hbm,
               xbuf, qbuf, kbuf, vbuf, wqbuf, wobuf, acc, obuf, xsem, ksem, vsem, qsem, osem, outsem):
        hbm = [(ax, akt, avt, awq, awo), (bx, bkt, bvt, bwq, bwo)]
        def x_cp(r, bi):
            return pltpu.make_async_copy(hbm[r][0].at[bi], xbuf.at[r, bi], xsem.at[r, bi])
        def k_cp(r, g, bi, slot):
            return pltpu.make_async_copy(hbm[r][1].at[bi, :, g], kbuf.at[slot, r], ksem.at[slot, r])
        def v_cp(r, g, bi, slot):
            return pltpu.make_async_copy(hbm[r][2].at[bi, :, g], vbuf.at[slot, r], vsem.at[slot, r])
        def wq_cp(r, g):
            return pltpu.make_async_copy(hbm[r][3].at[:, pl.ds(pl.multiple_of(g*W, 128), W)], wqbuf.at[g&1, r], qsem.at[g&1, r])
        def wo_cp(r, g):
            return pltpu.make_async_copy(hbm[r][4].at[g], wobuf.at[g&1, r], osem.at[g&1, r])
        def out_cp(bi):
            return pltpu.make_async_copy(obuf.at[bi], out_hbm.at[bi], outsem.at[bi])
        def start_kv(t, slot):
            if nodma: return
            g = t >> LB; bi = t & (NB-1)
            for r in range(2):
                k_cp(r, g, bi, slot).start()
                v_cp(r, g, bi, slot).start()
        def wait_kv(slot):
            if nodma: return
            for r in range(2):
                k_cp(r, 0, 0, slot).wait()
                v_cp(r, 0, 0, slot).wait()
        lo = lax.broadcasted_iota(jnp.int32, (HQ, 128), 1) < 64
        def sel(a, b): return jnp.where(lo, a, b)
        def rnd(a): return a.astype(bf16).astype(f32) if exact else a
        def qproj(r, bi, ws, jp):
            q = jnp.dot(xbuf[r, bi], wqbuf[ws, r, :, jp*384:(jp+1)*384], preferred_element_type=f32) * C
            res = []
            for bb in range(BB):
                t = q[bb*Sq:bb*Sq+HQ]; b = q[bb*Sq+HQ:(bb+1)*Sq]
                t0, t1, t2 = t[:, :128], t[:, 128:256], t[:, 256:]
                b0, b1, b2 = b[:, :128], b[:, 128:256], b[:, 256:]
                c = sel(t1, b1)
                cr = pltpu.roll(c, 64, 1)
                c = rnd(c)
                h0 = [sel(t0 - rnd(b0), t0), sel(b1 - c, b0), sel(b0, cr)]
                h1 = [sel(t2, t1 - c), sel(b2, b2 - rnd(t2)), sel(cr, t2)]
                res.append([jnp.concatenate(h, axis=0).astype(bf16) for h in (h0, h1)])
            return res
        def qstore(r, bi, jp, q):
            for bb in range(BB):
                for e in range(2): qbuf[r, bi, bb, 2*jp+e] = q[bb][e]
        for r in range(2):
            wq_cp(r, 0).start(); x_cp(r, 0).start()
        with ns("S_first"):
            for r in range(2): wq_cp(r, 0).wait()
        def pro(bi, c):
            with ns("S_xwait"):
                for r in range(2): x_cp(r, bi).wait()
            @pl.when(bi+1 < NB)
            def _():
                for r in range(2): x_cp(r, bi+1).start()
            @pl.when(bi == 0)
            def _():
                for r in range(2): wo_cp(r, 0).start()
            @pl.when(bi == 1)
            def _():
                for r in range(2): wq_cp(r, 1).start()
            for k in range(0 if nodma else 4):
                @pl.when(bi == min(NB-1, 2 + k))
                def _():
                    (k_cp if k % 2 == 0 else v_cp)(k//2, 0, 0, 0).start()
            @pl.when(bi == NB-1)
            def _():
                for s in range(1, NS-1): start_kv(s, s)
            with ns("S_pro"):
                for r in range(2):
                    for jp in range(G//2): qstore(r, bi, jp, qproj(r, bi, 0, jp))
                acc[bi] = jnp.zeros(acc.shape[1:], f32)
            return c
        lax.fori_loop(0, NB, pro, 0)

        def body(g, bi, slot, last):
            ws = g & 1
            units = [(r, bb, j) for r in range(2) for bb in range(BB) for j in range(G)]
            ps = {}; om = {}; os_ = {}; pend = []
            def blk(ref, lead, j, a, b):
                r0 = j*Dh
                if b == a+1: return ref[lead + (slice(r0+64*a, r0+64*a+128),)]
                return jnp.concatenate([ref[lead + (slice(r0+64*a, r0+64*a+64),)], ref[lead + (slice(r0+64*b, r0+64*b+64),)]], axis=0)
            def do_s(u):
                r, bb, j = u
                ws_ = [(0,1),(2,1),(0,2)] if j % 2 == 0 else [(1,0),(1,2),(0,2)]
                d = [jnp.dot(qbuf[r, bi, bb, j, i*HQ:(i+1)*HQ], blk(kbuf, (slot, r, bb), j, *ws_[i]), preferred_element_type=f32) for i in (2,0,1)]
                pp = []
                for s in (d[1]+d[0], d[2]+d[0]):
                    m = jnp.max(s, axis=-1, keepdims=True)
                    p = jnp.exp2(s-m)
                    l = jnp.sum(p, axis=-1, keepdims=True)
                    r0 = pl.reciprocal(l, approx=True)
                    pp.append(p * (r0*(2.0 - l*r0)))
                ps[u] = (pp[0].astype(bf16), pp[1].astype(bf16), (pp[0]-pp[1]).astype(bf16))
            def do_p(u):
                r, bb, j = u
                ws_ = [(0,1),(1,2),(0,2)] if j % 2 == 0 else [(1,0),(2,1),(2,0)]
                om[u] = [lax.dot_general(ps[u][i], blk(vbuf, (slot, r, bb), j, *ws_[i]), NT, preferred_element_type=f32) for i in range(3)]
                if j % 2 == 1:
                    X, Y, Z = om[(r, bb, j-1)]; X1, Y1, Z1 = om[u]
                    ta = jnp.concatenate([sel(X, Z+Y), sel(X-Z, Y)], axis=0)
                    tm = jnp.concatenate([sel(X1, X), pltpu.roll(sel(Y, Y1), 64, 1)], axis=0)
                    tb = jnp.concatenate([sel(Z1+Y1, X1), sel(Y1, X1-Z1)], axis=0)
                    os_[(r, bb, j//2)] = jnp.concatenate([ta, tm, tb], axis=1).astype(bf16)
            ocat = {}
            def do_o(r, c0, c1):
                if r not in ocat:
                    ocat[r] = jnp.concatenate([jnp.concatenate([os_[(r,bb,j)] for j in range(G//2)], axis=-1) for bb in range(BB)], axis=0)
                w = jnp.concatenate([wobuf[ws, r, jp*384+64*k:jp*384+64*k+64, c0:c1] for jp in range(G//2) for k in (0,2,4,1,5,3)], axis=0)
                res = acc[bi, :, r*D+c0:r*D+c1] + jnp.dot(ocat[r], w, preferred_element_type=f32)
                if last: obuf[bi, :, r*D+c0:r*D+c1] = res.astype(bf16)
                else: acc[bi, :, r*D+c0:r*D+c1] = res
            def do_q(r, jp, defer):
                q = qproj(r, bi, 1-ws, jp)
                if defer: pend.append((r, jp, q))
                else: qstore(r, bi, jp, q)
            def flush():
                for (r, jp, q) in pend: qstore(r, bi, jp, q)
                pend.clear()
            n = len(units); L = min(lag, n)
            fill = {i: [] for i in range(n+L+1)}
            P = functools.partial
            if inter == 0:
                if not last:
                    fill[n+L] += [P(do_q, r, jp, False) for r in range(2) for jp in range(G//2)]
                fill[n+L] += [P(do_o, 0, 0, D), P(do_o, 1, 0, D)]
            elif inter == 1:
                nA = n//2 + L + 1
                if not last:
                    qs = [P(do_q, r, jp, True) for r in range(2) for jp in range(G//2)]
                    for k, fn in enumerate(qs): fill[L + k*(nA-L)//len(qs)].append(fn)
                fill[nA+1].append(P(do_o, 0, 0, 256)); fill[nA+4].append(P(do_o, 0, 256, 640))
                fill[n+L] += [flush, P(do_o, 1, 0, D)]
            elif inter == 2:
                if not last:
                    qs = [P(do_q, r, jp, True) for r in range(2) for jp in range(G//2)]
                    for k, fn in enumerate(qs): fill[L + 1 + k*n//len(qs)].append(fn)
                fill[n+L] += [flush, P(do_o, 0, 0, D), P(do_o, 1, 0, D)]
            for i in range(n + L + 1):
                for ch in order:
                    if ch == "s" and i < n: do_s(units[i])
                    if ch == "f":
                        for fn in fill[i]: fn()
                    if ch == "p" and L <= i < n+L: do_p(units[i-L])

        def nxt(slot): return jnp.where(slot == NS-1, 0, slot+1)
        def prv(slot): return jnp.where(slot == 0, NS-1, slot-1)
        def group(g, slot):
            with ns("S_wwait"):
                for r in range(2):
                    wo_cp(r, g).wait(); wq_cp(r, g+1).wait()
            def step(bi, slot):
                t = (g << LB) + bi
                start_kv(t+NS-1, prv(slot))
                @pl.when(bi == 0)
                def _():
                    for r in range(2): wo_cp(r, g+1).start()
                    @pl.when(g+2 < NG)
                    def _():
                        for r in range(2): wq_cp(r, g+2).start()
                with ns("S_wait"): wait_kv(slot)
                with ns("S_body"): body(g, bi, slot, False)
                return nxt(slot)
            return lax.fori_loop(0, NB, step, slot)
        slot = lax.fori_loop(0, NG-1, group, 0)
        g = NG-1
        for r in range(2): wo_cp(r, g).wait()
        def lstep(bi, slot):
            t = (g << LB) + bi
            @pl.when(t+NS-1 < T)
            def _(): start_kv(t+NS-1, prv(slot))
            with ns("S_lwait"): wait_kv(slot)
            with ns("S_last"): body(g, bi, slot, True)
            out_cp(bi).start()
            return nxt(slot)
        lax.fori_loop(0, NB, lstep, slot)
        with ns("S_end"):
            for bi in range(NB): out_cp(bi).wait()

    def f(A_x, A_k, A_v, A_wq, A_wo, B_x, B_k, B_v, B_wq, B_wo):
        t = lambda a: jnp.swapaxes(a, 2, 3).reshape(NB, BB, NG, W, Sk)
        fx = lambda a: a.reshape(NB, M, D)
        fo = lambda a: a.reshape(NG, W, D)
        DMA = pltpu.SemaphoreType.DMA
        out = pl.pallas_call(
            kernel,
            in_specs=[pl.BlockSpec(memory_space=pl.ANY)]*10,
            out_specs=pl.BlockSpec(memory_space=pl.ANY),
            out_shape=jax.ShapeDtypeStruct((NB, M, 2*D), bf16),
            scratch_shapes=[
                pltpu.VMEM((2, NB, M, D), bf16),
                pltpu.VMEM((2, NB, BB, G, 3*HQ, 128), bf16),
                pltpu.VMEM((NS, 2, BB, W, Sk), bf16),
                pltpu.VMEM((NS, 2, BB, W, Sk), bf16),
                pltpu.VMEM((2, 2, D, W), bf16),
                pltpu.VMEM((2, 2, W, D), bf16),
                pltpu.VMEM((NB, M, 2*D), f32),
                pltpu.VMEM((NB, M, 2*D), bf16),
                DMA((2, NB)), DMA((NS, 2)), DMA((NS, 2)), DMA((2, 2)), DMA((2, 2)), DMA((NB,)),
            ],
            compiler_params=pltpu.CompilerParams(vmem_limit_bytes=vmem*1024*1024, flags=flags, disable_bounds_checks=True),
            name="attn_v7",
        )(fx(A_x), t(A_k), t(A_v), A_wq, fo(A_wo), fx(B_x), t(B_k), t(B_v), B_wq, fo(B_wo))
        return out.reshape(B, Sq, 2*D)
    return f


_impl = build(lag=2)


@jax.jit
def pallas_concat_heads__gqa_block_cached__mha_block_cached__near_ridge_kernel(
    A_x, A_k_cache, A_v_cache, A_wq, A_wo, B_x, B_k_cache, B_v_cache, B_wq, B_wo
):
    return _impl(A_x, A_k_cache, A_v_cache, A_wq, A_wo, B_x, B_k_cache, B_v_cache, B_wq, B_wo)
```

```python
import functools, contextlib
import jax, jax.numpy as jnp, numpy as np
from jax import lax
from jax.experimental import pallas as pl
from jax.experimental.pallas import tpu as pltpu

B,Sq,D,H,Sk,Dh = 16,160,640,32,512,192
C = float(Dh**-0.5 * np.log2(np.e))
NT = (((1,),(1,)),((),()))
f32 = jnp.float32; bf16 = jnp.bfloat16
HQ = Sq//2

def build(G=4, BB=2, vmem=110, lag=2, flags=None, NS=3, inter=0, order="sfp", prof=False, exact=True, nodma=False, rg=0, qw=384, ow=128, odelay=1, f0=1, L_={}):
    PM = dict(lag=lag, inter=inter, order=order, rg=rg, qw=qw, ow=ow, odelay=odelay, f0=f0); PL = dict(PM, **L_)
    ns = (lambda n: jax.named_scope(n)) if prof else (lambda n: contextlib.nullcontext())
    NG = H//G; NB = B//BB; T = NG*NB; M = BB*Sq; W = G*Dh
    assert NB & (NB-1) == 0
    LB = NB.bit_length()-1
    def kernel(ax, akt, avt, awq, awo, bx, bkt, bvt, bwq, bwo, out_hbm,
               xbuf, qbuf, kbuf, vbuf, wqbuf, wobuf, acc, obuf, xsem, ksem, vsem, qsem, osem, outsem):
        hbm = [(ax, akt, avt, awq, awo), (bx, bkt, bvt, bwq, bwo)]
        def x_cp(r, bi):
            return pltpu.make_async_copy(hbm[r][0].at[bi], xbuf.at[r, bi], xsem.at[r, bi])
        def k_cp(r, g, bi, slot):
            return pltpu.make_async_copy(hbm[r][1].at[bi, :, g], kbuf.at[slot, r], ksem.at[slot, r])
        def v_cp(r, g, bi, slot):
            return pltpu.make_async_copy(hbm[r][2].at[bi, :, g], vbuf.at[slot, r], vsem.at[slot, r])
        def wq_cp(r, g):
            return pltpu.make_async_copy(hbm[r][3].at[:, pl.ds(pl.multiple_of(g*W, 128), W)], wqbuf.at[g&1, r], qsem.at[g&1, r])
        def wo_cp(r, g):
            return pltpu.make_async_copy(hbm[r][4].at[g], wobuf.at[g&1, r], osem.at[g&1, r])
        def out_cp(bi):
            return pltpu.make_async_copy(obuf.at[bi], out_hbm.at[bi], outsem.at[bi])
        def start_kv(t, slot):
            if nodma: return
            g = t >> LB; bi = t & (NB-1)
            for r in range(2):
                k_cp(r, g, bi, slot).start()
                v_cp(r, g, bi, slot).start()
        def wait_kv(slot):
            if nodma: return
            for r in range(2):
                k_cp(r, 0, 0, slot).wait()
                v_cp(r, 0, 0, slot).wait()
        lo = lax.broadcasted_iota(jnp.int32, (HQ, 128), 1) < 64
        def sel(a, b): return jnp.where(lo, a, b)
        def rnd(a): return a.astype(bf16).astype(f32) if exact else a
        def qproj(r, bi, ws, jp):
            return qfin(jnp.dot(xbuf[r, bi], wqbuf[ws, r, :, jp*384:(jp+1)*384], preferred_element_type=f32))
        def qfin(q):
            q = q * C
            res = []
            for bb in range(BB):
                t = q[bb*Sq:bb*Sq+HQ]; b = q[bb*Sq+HQ:(bb+1)*Sq]
                t0, t1, t2 = t[:, :128], t[:, 128:256], t[:, 256:]
                b0, b1, b2 = b[:, :128], b[:, 128:256], b[:, 256:]
                c = sel(t1, b1)
                cr = pltpu.roll(c, 64, 1)
                c = rnd(c)
                h0 = [sel(t0 - rnd(b0), t0), sel(b1 - c, b0), sel(b0, cr)]
                h1 = [sel(t2, t1 - c), sel(b2, b2 - rnd(t2)), sel(cr, t2)]
                res.append([jnp.concatenate(h, axis=0).astype(bf16) for h in (h0, h1)])
            return res
        def qstore(r, bi, jp, q):
            for bb in range(BB):
                for e in range(2): qbuf[r, bi, bb, 2*jp+e] = q[bb][e]
        for r in range(2):
            wq_cp(r, 0).start(); x_cp(r, 0).start()
        with ns("S_first"):
            for r in range(2): wq_cp(r, 0).wait()
        def pro(bi, c):
            with ns("S_xwait"):
                for r in range(2): x_cp(r, bi).wait()
            @pl.when(bi+1 < NB)
            def _():
                for r in range(2): x_cp(r, bi+1).start()
            @pl.when(bi == 0)
            def _():
                for r in range(2): wo_cp(r, 0).start()
            @pl.when(bi == 1)
            def _():
                for r in range(2): wq_cp(r, 1).start()
            for k in range(0 if nodma else 4):
                @pl.when(bi == min(NB-1, 2 + k))
                def _():
                    (k_cp if k % 2 == 0 else v_cp)(k//2, 0, 0, 0).start()
            @pl.when(bi == NB-1)
            def _():
                for s in range(1, NS-1): start_kv(s, s)
            with ns("S_pro"):
                for r in range(2):
                    for jp in range(G//2): qstore(r, bi, jp, qproj(r, bi, 0, jp))
                acc[bi] = jnp.zeros(acc.shape[1:], f32)
            return c
        lax.fori_loop(0, NB, pro, 0)

        def body(g, bi, slot, last):
            ws = g & 1
            lag, inter, order, rg, qw, ow, odelay, f0 = (PL if last else PM).values()
            units = [(r, bb, j) for r in range(2) for bb in range(BB) for j in range(G)]
            ps = {}; om = {}; os_ = {}; pend = []
            def blk(ref, lead, j, a, b):
                r0 = j*Dh
                if b == a+1: return ref[lead + (slice(r0+64*a, r0+64*a+128),)]
                return jnp.concatenate([ref[lead + (slice(r0+64*a, r0+64*a+64),)], ref[lead + (slice(r0+64*b, r0+64*b+64),)]], axis=0)
            def do_s(u):
                r, bb, j = u
                ws_ = [(0,1),(2,1),(0,2)] if j % 2 == 0 else [(1,0),(1,2),(0,2)]
                d = [jnp.dot(qbuf[r, bi, bb, j, i*HQ:(i+1)*HQ], blk(kbuf, (slot, r, bb), j, *ws_[i]), preferred_element_type=f32) for i in (2,0,1)]
                def sm(s):
                    m = jnp.max(s, axis=-1, keepdims=True)
                    p = jnp.exp2(s-m)
                    l = jnp.sum(p, axis=-1, keepdims=True)
                    r0 = pl.reciprocal(l, approx=True)
                    return p * (r0*(2.0 - l*r0))
                if rg == 0:
                    pp = [sm(d[1]+d[0]), sm(d[2]+d[0])]
                    ps[u] = (pp[0].astype(bf16), pp[1].astype(bf16), (pp[0]-pp[1]).astype(bf16))
                else:
                    o3 = [[], [], []]
                    for i0 in range(0, HQ, rg):
                        sl = slice(i0, i0+rg)
                        a = sm(d[1][sl]+d[0][sl]); b = sm(d[2][sl]+d[0][sl])
                        o3[0].append(a.astype(bf16)); o3[1].append(b.astype(bf16)); o3[2].append((a-b).astype(bf16))
                    ps[u] = tuple(jnp.concatenate(o, axis=0) for o in o3)
            def do_p(u):
                r, bb, j = u
                ws_ = [(0,1),(1,2),(0,2)] if j % 2 == 0 else [(1,0),(2,1),(2,0)]
                om[u] = [lax.dot_general(ps[u][i], blk(vbuf, (slot, r, bb), j, *ws_[i]), NT, preferred_element_type=f32) for i in range(3)]
                if j % 2 == 1:
                    X, Y, Z = om[(r, bb, j-1)]; X1, Y1, Z1 = om[u]
                    ta = jnp.concatenate([sel(X, Z+Y), sel(X-Z, Y)], axis=0)
                    tm = jnp.concatenate([sel(X1, X), pltpu.roll(sel(Y, Y1), 64, 1)], axis=0)
                    tb = jnp.concatenate([sel(Z1+Y1, X1), sel(Y1, X1-Z1)], axis=0)
                    os_[(r, bb, j//2)] = jnp.concatenate([ta, tm, tb], axis=1).astype(bf16)
            ocat = {}
            def do_o(r, c0, c1):
                if r not in ocat:
                    ocat[r] = jnp.concatenate([jnp.concatenate([os_[(r,bb,j)] for j in range(G//2)], axis=-1) for bb in range(BB)], axis=0)
                w = jnp.concatenate([wobuf[ws, r, jp*384+64*k:jp*384+64*k+64, c0:c1] for jp in range(G//2) for k in (0,2,4,1,5,3)], axis=0)
                res = acc[bi, :, r*D+c0:r*D+c1] + jnp.dot(ocat[r], w, preferred_element_type=f32)
                if last: obuf[bi, :, r*D+c0:r*D+c1] = res.astype(bf16)
                else: acc[bi, :, r*D+c0:r*D+c1] = res
            def do_o2(r, bb, c0, c1):
                if (r, bb) not in ocat:
                    ocat[(r, bb)] = jnp.concatenate([os_[(r,bb,j)] for j in range(G//2)], axis=-1)
                w = jnp.concatenate([wobuf[ws, r, jp*384+64*k:jp*384+64*k+64, c0:c1] for jp in range(G//2) for k in (0,2,4,1,5,3)], axis=0)
                rows = slice(bb*Sq, (bb+1)*Sq)
                res = acc[bi, rows, r*D+c0:r*D+c1] + jnp.dot(ocat[(r, bb)], w, preferred_element_type=f32)
                if last: obuf[bi, rows, r*D+c0:r*D+c1] = res.astype(bf16)
                else: acc[bi, rows, r*D+c0:r*D+c1] = res
            def do_q(r, jp, defer):
                q = qproj(r, bi, 1-ws, jp)
                if defer: pend.append((r, jp, q))
                else: qstore(r, bi, jp, q)
            qc = {}
            def do_qc(r, jp, c0, c1):
                qc.setdefault((r, jp), []).append(jnp.dot(xbuf[r, bi], wqbuf[1-ws, r, :, jp*384+c0:jp*384+c1], preferred_element_type=f32))
                if c1 == 384: pend.append((r, jp, qfin(jnp.concatenate(qc[(r, jp)], axis=1))))
            def flush():
                for (r, jp, q) in pend: qstore(r, bi, jp, q)
                pend.clear()
            n = len(units); L = min(lag, n)
            fill = {i: [] for i in range(n+L+1)}
            P = functools.partial
            if inter == 0:
                if not last:
                    fill[n+L] += [P(do_q, r, jp, False) for r in range(2) for jp in range(G//2)]
                fill[n+L] += [P(do_o, 0, 0, D), P(do_o, 1, 0, D)]
            elif inter == 1:
                nA = n//2 + L + 1
                if not last:
                    qs = [P(do_q, r, jp, True) for r in range(2) for jp in range(G//2)]
                    for k, fn in enumerate(qs): fill[L + k*(nA-L)//len(qs)].append(fn)
                fill[nA+1].append(P(do_o, 0, 0, 256)); fill[nA+4].append(P(do_o, 0, 256, 640))
                fill[n+L] += [flush, P(do_o, 1, 0, D)]
            elif inter == 3:
                nA = n//2 + L + 1
                if not last:
                    qs = [P(do_qc, r, jp, c, min(c+qw, 384)) for r in range(2) for jp in range(G//2) for c in range(0, 384, qw)]
                    for k, fn in enumerate(qs): fill[1 + k*(nA-1)//len(qs)].append(fn)
                osl = [P(do_o, 0, c, c+128) for c in range(0, D, 128)]
                for k, fn in enumerate(osl): fill[nA + k*(n+L+1-nA)//len(osl)].append(fn)
                fill[n+L] += [flush, P(do_o, 1, 0, D)]
            elif inter == 4:
                if not last:
                    qs = [P(do_qc, r, jp, c, min(c+qw, 384)) for r in range(2) for jp in range(G//2) for c in range(0, 384, qw)]
                    for k, fn in enumerate(qs): fill[1 + k*(n+L-1)//len(qs)].append(fn)
                fill[n+L] += [flush, P(do_o, 0, 0, D), P(do_o, 1, 0, D)]
            elif inter == 5:
                qs = [] if last else [(P(do_qc, r, jp, c, min(c+qw, 384)), (min(c+qw, 384)-c)//128*5*M/4) for r in range(2) for jp in range(G//2) for c in range(0, 384, qw)]
                osl = []
                for k in range(2*BB):
                    for c in range(0, D, ow):
                        osl.append(((k+1)*G - 1 + L + odelay, P(do_o2, k//BB, k%BB, c, min(c+ow, D)), (min(c+ow, D)-c)//128*(W//128)*Sq/4))
                tot = sum(w for _, w in qs) + sum(w for a, _, w in osl if a < n+L)
                nsl = n + L - f0
                done = 0
                for i in range(f0, n+L):
                    tgt = tot*(i-f0+1)/nsl
                    while done < tgt - 1:
                        navail = sum(w for a, _, w in osl if a <= i)
                        if osl and osl[0][0] <= i and (not last or done + osl[0][2]/2 <= tgt or navail > 5*ow//128*(W//128)*Sq/4/G*((osl[0][0]-L-odelay+1) + G + L + odelay - 1 - i)):
                            _, fn, w = osl.pop(0)
                        elif qs: fn, w = qs.pop(0)
                        else: break
                        fill[i].append(fn); done += w
                fill[n+L] += [fn for fn, _ in qs] + [flush] + [fn for _, fn, _ in osl]
            elif inter == 2:
                if not last:
                    qs = [P(do_q, r, jp, True) for r in range(2) for jp in range(G//2)]
                    for k, fn in enumerate(qs): fill[L + 1 + k*n//len(qs)].append(fn)
                fill[n+L] += [flush, P(do_o, 0, 0, D), P(do_o, 1, 0, D)]
            for i in range(n + L + 1):
                for ch in order:
                    if ch == "s" and i < n: do_s(units[i])
                    if ch == "f":
                        for fn in fill[i]: fn()
                    if ch == "p" and L <= i < n+L: do_p(units[i-L])

        def nxt(slot): return jnp.where(slot == NS-1, 0, slot+1)
        def prv(slot): return jnp.where(slot == 0, NS-1, slot-1)
        def group(g, slot):
            with ns("S_wwait"):
                for r in range(2):
                    wo_cp(r, g).wait(); wq_cp(r, g+1).wait()
            def step(bi, slot):
                t = (g << LB) + bi
                start_kv(t+NS-1, prv(slot))
                @pl.when(bi == 0)
                def _():
                    for r in range(2): wo_cp(r, g+1).start()
                    @pl.when(g+2 < NG)
                    def _():
                        for r in range(2): wq_cp(r, g+2).start()
                with ns("S_wait"): wait_kv(slot)
                with ns("S_body"): body(g, bi, slot, False)
                return nxt(slot)
            return lax.fori_loop(0, NB, step, slot)
        slot = lax.fori_loop(0, NG-1, group, 0)
        g = NG-1
        for r in range(2): wo_cp(r, g).wait()
        def lstep(bi, slot):
            t = (g << LB) + bi
            @pl.when(t+NS-1 < T)
            def _(): start_kv(t+NS-1, prv(slot))
            with ns("S_lwait"): wait_kv(slot)
            with ns("S_last"): body(g, bi, slot, True)
            out_cp(bi).start()
            return nxt(slot)
        lax.fori_loop(0, NB, lstep, slot)
        with ns("S_end"):
            for bi in range(NB): out_cp(bi).wait()

    def f(A_x, A_k, A_v, A_wq, A_wo, B_x, B_k, B_v, B_wq, B_wo):
        t = lambda a: jnp.swapaxes(a, 2, 3).reshape(NB, BB, NG, W, Sk)
        fx = lambda a: a.reshape(NB, M, D)
        fo = lambda a: a.reshape(NG, W, D)
        DMA = pltpu.SemaphoreType.DMA
        out = pl.pallas_call(
            kernel,
            in_specs=[pl.BlockSpec(memory_space=pl.ANY)]*10,
            out_specs=pl.BlockSpec(memory_space=pl.ANY),
            out_shape=jax.ShapeDtypeStruct((NB, M, 2*D), bf16),
            scratch_shapes=[
                pltpu.VMEM((2, NB, M, D), bf16),
                pltpu.VMEM((2, NB, BB, G, 3*HQ, 128), bf16),
                pltpu.VMEM((NS, 2, BB, W, Sk), bf16),
                pltpu.VMEM((NS, 2, BB, W, Sk), bf16),
                pltpu.VMEM((2, 2, D, W), bf16),
                pltpu.VMEM((2, 2, W, D), bf16),
                pltpu.VMEM((NB, M, 2*D), f32),
                pltpu.VMEM((NB, M, 2*D), bf16),
                DMA((2, NB)), DMA((NS, 2)), DMA((NS, 2)), DMA((2, 2)), DMA((2, 2)), DMA((NB,)),
            ],
            compiler_params=pltpu.CompilerParams(vmem_limit_bytes=vmem*1024*1024, flags=flags, disable_bounds_checks=True),
            name="attn_v7",
        )(fx(A_x), t(A_k), t(A_v), A_wq, fo(A_wo), fx(B_x), t(B_k), t(B_v), B_wq, fo(B_wo))
        return out.reshape(B, Sq, 2*D)
    return f


_impl = build(inter=5, rg=16, qw=128, order='spf', L_=dict(order='sfp'))


@jax.jit
def pallas_concat_heads__gqa_block_cached__mha_block_cached__near_ridge_kernel(
    A_x, A_k_cache, A_v_cache, A_wq, A_wo, B_x, B_k_cache, B_v_cache, B_wq, B_wo
):
    return _impl(A_x, A_k_cache, A_v_cache, A_wq, A_wo, B_x, B_k_cache, B_v_cache, B_wq, B_wo)
```

```python
import functools, contextlib
import jax, jax.numpy as jnp, numpy as np
from jax import lax
from jax.experimental import pallas as pl
from jax.experimental.pallas import tpu as pltpu

B,Sq,D,H,Sk,Dh = 16,160,640,32,512,192
C = float(Dh**-0.5 * np.log2(np.e))
NT = (((1,),(1,)),((),()))
f32 = jnp.float32; bf16 = jnp.bfloat16
HQ = Sq//2
G = 4; BB = 2
NG = H//G; NB = B//BB; NBLK = NG*NB; M = BB*Sq; W = G*Dh

def build(U=2, DQ=10, NS=3, vmem=120, flags=None, prof=False, nodma=False, NP=8,
          lag=1, order="spf", rg=16, qw=128, ow=128, odelay=1, f0=0, pmode=2, rnd_=True, so=(2,0,1), po=(0,1,2), seed=0, L_={}, zmode=1):
    ns = (lambda n: jax.named_scope(n)) if prof else (lambda n: contextlib.nullcontext())
    PM = dict(lag=lag, order=order, rg=rg, qw=qw, ow=ow, odelay=odelay, f0=f0, so=so, po=po, seed=seed); PL = dict(PM, **L_)
    NT_ = NBLK//U; TM = (NBLK-DQ)//U; SPG = NB//U
    assert DQ % 2 == 0 and NB <= DQ <= 2*NB
    def kernel(ax, akt, avt, awq, awo, bx, bkt, bvt, bwq, bwo, out_hbm,
               xbuf, qbuf, kbuf, vbuf, wqbuf, wobuf, acc, obuf, pbuf, xsem, kvsem, qsem, osem, outsem, fsem):
        hbm = [(ax, akt, avt, awq, awo), (bx, bkt, bvt, bwq, bwo)]
        cp = pltpu.make_async_copy
        def x_cp(r, k):
            return cp(hbm[r][0].at[pl.ds(2*k, 2)], xbuf.at[r, pl.ds(2*k, 2)], xsem.at[r*(NB//2)+k])
        def x_wait(i):
            cp(ax.at[pl.ds(0, 2)], xbuf.at[0, pl.ds(0, 2)], xsem.at[i]).wait()
        def kv_cps(t, slot):
            g = lax.shift_right_logical(t, SPG.bit_length()-1); s = t & (SPG-1)
            return [cp(hbm[r][1+e].at[s, :, g], (kbuf, vbuf)[e].at[slot, r], kvsem.at[slot, 2*r+e]) for r in range(2) for e in range(2)]
        def wq_cp(r, g):
            return cp(hbm[r][3].at[:, pl.ds(pl.multiple_of(g*W, 128), W)], wqbuf.at[g&1, r], qsem.at[g&1, r])
        def wo_cp(r, g):
            return cp(hbm[r][4].at[g], wobuf.at[g&1, r], osem.at[g&1, r])
        def out_cp(bi):
            return cp(obuf.at[bi], out_hbm.at[bi], outsem.at[bi])
        def start_kv(t, slot):
            if nodma: return
            for c in kv_cps(t, slot): c.start()
        def wait_kv(slot):
            if nodma: return
            for c in kv_cps(0, slot): c.wait()
        lo = lax.broadcasted_iota(jnp.int32, (HQ, 128), 1) < 64
        def sel(a, b): return jnp.where(lo, a, b)
        def rnd(a): return a.astype(bf16).astype(f32) if rnd_ else a
        def qdot(r, bi, ws, c0, c1):
            return jnp.dot(xbuf[r, bi], wqbuf[ws, r, :, c0:c1], preferred_element_type=f32)
        def qfin(q):
            q = q * C
            res = []
            for bb in range(BB):
                t = q[bb*Sq:bb*Sq+HQ]; b = q[bb*Sq+HQ:(bb+1)*Sq]
                t0, t1, t2 = t[:, :128], t[:, 128:256], t[:, 256:]
                b0, b1, b2 = b[:, :128], b[:, 128:256], b[:, 256:]
                c = sel(t1, b1)
                cr = pltpu.roll(c, 64, 1)
                c = rnd(c)
                h0 = [sel(t0 - rnd(b0), t0), sel(b1 - c, b0), sel(b0, cr)]
                h1 = [sel(t2, t1 - c), sel(b2, b2 - rnd(t2)), sel(cr, t2)]
                res.append([jnp.concatenate(h, axis=0).astype(bf16) for h in (h0, h1)])
            return res
        def qstore(qs, r, jp, q):
            for bb in range(BB):
                for e in range(2): qbuf[qs, r, bb, 2*jp+e] = q[bb][e]
        def qpair(qs, r, bi, ws, jp):
            qstore(qs, r, jp, qfin(qdot(r, bi, ws, jp*384, (jp+1)*384)))
        first = [cp(awq.at[:, 0:384], wqbuf.at[0, 0, :, 0:384], fsem.at[0]), cp(ax.at[0], xbuf.at[0, 0], fsem.at[1]),
                 cp(awq.at[:, 384:768], wqbuf.at[0, 0, :, 384:768], fsem.at[2]), cp(ax.at[1], xbuf.at[0, 1], fsem.at[3])]
        for c in first: c.start()
        for k in range(1, NB//2): x_cp(0, k).start()
        def zero(i, c):
            acc[i] = jnp.zeros(acc.shape[1:], f32)
            return c
        if zmode == 0: lax.fori_loop(0, 3, zero, 0)
        with ns("S_first"):
            first[0].wait(); first[1].wait()
        qpair(0, 0, 0, 0, 0)
        wq_cp(1, 0).start()
        for k in range(NB//2): x_cp(1, k).start()
        for r in range(2): wq_cp(r, 1).start()
        first[2].wait(); first[3].wait()
        qpair(0, 0, 0, 0, 1); qpair(1, 0, 1, 0, 0); qpair(1, 0, 1, 0, 1)
        start_kv(0, 0)
        for r in range(2): wo_cp(r, 0).start()
        def pro(i, c):
            late = i >= NB
            r = jnp.where(late, i & 1, lax.shift_right_logical(i, 2))
            k = jnp.where(late, lax.shift_right_logical(i-NB, 1), i & 3)
            ws = late.astype(jnp.int32)
            with ns("S_xwait"):
                @pl.when(i < NB)
                def _(): x_wait(i)
                @pl.when(i == NB//2)
                def _():
                    wq_cp(1, 0).wait()
                    for s in range(1, NS-1): start_kv(s, s)
                @pl.when(i == min(NB, DQ-1))
                def _():
                    for rr in range(2): wq_cp(rr, 1).wait()
            with ns("S_pro"):
                for h in range(2):
                    for jp in range(G//2):
                        qpair(ws*NB + 2*k + h, r, 2*k + h, ws, jp)
                        if zmode == 0 and 2*h+jp < 3:
                            zr = [(0, 104), (104, 208), (208, 320)][2*h+jp]
                            acc[jnp.minimum(i+2, NB-1), zr[0]:zr[1]] = jnp.zeros((zr[1]-zr[0], 2*D), f32)
            return c
        lax.fori_loop(1, DQ, pro, 0)

        def body(blocks, slot, last):
            lag, order, rg, qw, ow, odelay, f0, so, po, seed = (PL if last else PM).values()
            nb = len(blocks)
            bis = [n & (NB-1) for n, _, _ in blocks]
            wos = lax.shift_right_logical(blocks[0][0], 3) & 1
            nq = blocks[0][0] + DQ
            wqs = lax.shift_right_logical(nq, 3) & 1
            units = [(h, r, bb, j) for h in range(nb) for r in range(2) for bb in range(BB) for j in range(G)]
            om = {}; os_ = {}; pend = []; qc = {}; ocat = {}
            def blk(ref, u, a, b):
                h, r, bb, j = u
                lead = (slot, r, blocks[h][2] + bb); r0 = j*Dh
                if b == a+1: return ref[lead + (slice(r0+64*a, r0+64*a+128),)]
                return jnp.concatenate([ref[lead + (slice(r0+64*a, r0+64*a+64),)], ref[lead + (slice(r0+64*b, r0+64*b+64),)]], axis=0)
            def sm(s):
                m = jnp.max(s, axis=-1, keepdims=True)
                p = jnp.exp2(s-m)
                l = jnp.sum(p, axis=-1, keepdims=True)
                r0 = pl.reciprocal(l, approx=True)
                return p * (r0*(2.0 - l*r0))
            def do_s(ui):
                u = units[ui]; h, r, bb, j = u
                ws_ = [(0,1),(2,1),(0,2)] if j % 2 == 0 else [(1,0),(1,2),(0,2)]
                d = {i: jnp.dot(qbuf[blocks[h][1], r, bb, j, i*HQ:(i+1)*HQ], blk(kbuf, u, *ws_[i]), preferred_element_type=f32) for i in so}
                k = ui % NP
                for i0 in range(0, HQ, rg):
                    sl = slice(i0, i0+rg)
                    a = sm(d[0][sl]+d[2][sl]); b = sm(d[1][sl]+d[2][sl])
                    for e, z in enumerate((a, b, a-b)):
                        if pmode == 1: pbuf[k, e, sl] = z.astype(bf16)
                        else:
                            for c in range(4): pbuf[k, e, c, sl] = z[:, c*128:(c+1)*128].astype(bf16)
            def do_p(ui):
                u = units[ui]; h, r, bb, j = u
                ws_ = [(0,1),(1,2),(0,2)] if j % 2 == 0 else [(1,0),(2,1),(2,0)]
                o = {}
                for i in po:
                    vv = blk(vbuf, u, *ws_[i])
                    if pmode == 1: o[i] = lax.dot_general(pbuf[ui % NP, i], vv, NT, preferred_element_type=f32)
                    else:
                        dd = [lax.dot_general(pbuf[ui % NP, i, c], vv[:, c*128:(c+1)*128], NT, preferred_element_type=f32) for c in range(4)]
                        o[i] = (dd[0]+dd[1])+(dd[2]+dd[3])
                om[ui] = [o[i] for i in range(3)]
                if j % 2 == 1:
                    X, Y, Z = om[ui-1]; X1, Y1, Z1 = om[ui]
                    ta = jnp.concatenate([sel(X, Z+Y), sel(X-Z, Y)], axis=0)
                    tm = jnp.concatenate([sel(X1, X), pltpu.roll(sel(Y, Y1), 64, 1)], axis=0)
                    tb = jnp.concatenate([sel(Z1+Y1, X1), sel(Y1, X1-Z1)], axis=0)
                    os_[(h, r, bb, j//2)] = jnp.concatenate([ta, tm, tb], axis=1)
            def do_o(h, r, bb, c0, c1):
                if (h, r, bb) not in ocat:
                    ocat[(h, r, bb)] = jnp.concatenate([os_[(h, r, bb, jp)] for jp in range(G//2)], axis=-1).astype(bf16)
                w = jnp.concatenate([wobuf[wos, r, jp*384+64*k:jp*384+64*k+64, c0:c1] for jp in range(G//2) for k in (0,2,4,1,5,3)], axis=0)
                idx = (bis[h], slice(bb*Sq, (bb+1)*Sq), slice(r*D+c0, r*D+c1))
                prev = acc[idx]
                if zmode == 1 and not last: prev = jnp.where(jnp.full(prev.shape, blocks[0][0], jnp.int32) >= NB, prev, 0.0)
                res = prev + jnp.dot(ocat[(h, r, bb)], w, preferred_element_type=f32)
                if last: obuf[idx] = res.astype(bf16)
                if not last or DQ > NB: acc[idx] = res
            def do_q(h, r, jp, c0, c1):
                qc.setdefault((h, r, jp), []).append(qdot(r, (nq + h) & (NB-1), wqs, jp*384+c0, jp*384+c1))
                if c1 == 384: pend.append((blocks[h][1], r, jp, qfin(jnp.concatenate(qc[(h, r, jp)], axis=1))))
            def flush():
                for a in pend: qstore(*a)
                pend.clear()
            n = len(units); L = lag; P = functools.partial
            fill = {i: [] for i in range(n+L+1)}
            qs = [] if last else [(P(do_q, h, r, jp, c, min(c+qw, 384)), (min(c+qw, 384)-c)//128*5*M/4)
                                  for h in range(nb) for r in range(2) for jp in range(G//2) for c in range(0, 384, qw)]
            osl = [((k+1)*G - 1 + L + odelay, P(do_o, units[k*G][0], units[k*G][1], units[k*G][2], c, min(c+ow, D)), (min(c+ow, D)-c)//128*6*Sq/4)
                   for k in range(n//G) for c in range(0, D, ow)]
            tot = sum(w for _, w in qs) + sum(w for a, _, w in osl if a < n+L)
            nsl = n + L - f0; done = 0
            rs = np.random.RandomState(seed)
            for i in range(f0, n+L):
                tgt = tot*(i-f0+1)/nsl + (rs.uniform(-200, 200) if seed else 0)
                cnt = 0
                while done < tgt - 1:
                    nav = sum(1 for a, _, w in osl if a <= i)
                    left = G - (i - L - odelay + 1) % G
                    useo = nav > 0 and ((cnt < -(-nav//left)) if last else True)
                    if useo: _, fn, w = osl.pop(0); cnt += 1
                    elif qs: fn, w = qs.pop(0)
                    else: break
                    fill[i].append(fn); done += w
            fill[n+L] += [fn for fn, _ in qs] + [flush] + [fn for _, fn, _ in osl]
            for i in range(n + L + 1):
                fl = fill[i]; nf = order.count("f"); kf = 0
                for ch in order:
                    if ch == "s" and i < n: do_s(i)
                    if ch == "f":
                        for fn in fl[-(-kf*len(fl)//nf):-(-(kf+1)*len(fl)//nf)]: fn()
                        kf += 1
                    if ch == "p" and L <= i < n+L: do_p(i-L)

        def nxt(s, n): return jnp.where(s == n-1, 0, s+1)
        def prv(s, n): return jnp.where(s == 0, n-1, s-1)
        def wo_stage(t):
            @pl.when((t & (SPG-1)) == 0)
            def _():
                g = lax.shift_right_logical(t, SPG.bit_length()-1)
                for r in range(2): wo_cp(r, g).wait()
                @pl.when(g+1 < NG)
                def _():
                    for r in range(2): wo_cp(r, g+1).start()
        if DQ > NB:
            for r in range(2): wq_cp(r, 2).start()
        def step(t, c):
            slot, q = c
            start_kv(t+NS-1, prv(slot, NS))
            wo_stage(t)
            tq = t + DQ//U
            @pl.when((tq & (SPG-1)) == 0)
            def _():
                g = lax.shift_right_logical(tq, SPG.bit_length()-1)
                @pl.when(g > 1)
                def _():
                    for r in range(2): wq_cp(r, g).wait()
                @pl.when(g+1 < NG)
                def _():
                    for r in range(2): wq_cp(r, g+1).start()
            with ns("S_wait"): wait_kv(slot)
            with ns("S_body"): body([(t*U+h, q*U+h, h*BB) for h in range(U)], slot, False)
            return nxt(slot, NS), nxt(q, DQ//U)
        slot, q = lax.fori_loop(0, TM, step, (0, 0))
        def lstep(n, c):
            slot, q = c
            t = n >> (U-1); h = n & (U-1)
            @pl.when(h == 0)
            def _():
                @pl.when(t+NS-1 < NT_)
                def _(): start_kv(t+NS-1, prv(slot, NS))
                wo_stage(t)
                with ns("S_lwait"): wait_kv(slot)
            with ns("S_last"): body([(n, q, h*BB)], slot, True)
            @pl.when(n >= NBLK-NB)
            def _(): out_cp(n & (NB-1)).start()
            return jnp.where(h == U-1, nxt(slot, NS), slot), nxt(q, DQ)
        lax.fori_loop(NBLK-DQ, NBLK, lstep, (slot, q*U))
        with ns("S_end"):
            for bi in range(NB): out_cp(bi).wait()

    def f(A_x, A_k, A_v, A_wq, A_wo, B_x, B_k, B_v, B_wq, B_wo):
        t = lambda a: jnp.swapaxes(a, 2, 3).reshape(SPG, U*BB, NG, W, Sk)
        fx = lambda a: a.reshape(NB, M, D)
        fo = lambda a: a.reshape(NG, W, D)
        DMA = pltpu.SemaphoreType.DMA
        out = pl.pallas_call(
            kernel,
            in_specs=[pl.BlockSpec(memory_space=pl.ANY)]*10,
            out_specs=pl.BlockSpec(memory_space=pl.ANY),
            out_shape=jax.ShapeDtypeStruct((NB, M, 2*D), bf16),
            scratch_shapes=[
                pltpu.VMEM((2, NB, M, D), bf16),
                pltpu.VMEM((DQ, 2, BB, G, 3*HQ, 128), bf16),
                pltpu.VMEM((NS, 2, U*BB, W, Sk), bf16),
                pltpu.VMEM((NS, 2, U*BB, W, Sk), bf16),
                pltpu.VMEM((2, 2, D, W), bf16),
                pltpu.VMEM((2, 2, W, D), bf16),
                pltpu.VMEM((NB, M, 2*D), f32),
                pltpu.VMEM((NB, M, 2*D), bf16),
                pltpu.VMEM((NP, 3, HQ, Sk) if pmode < 2 else (NP, 3, 4, HQ, 128), bf16),
                DMA((NB,)), DMA((NS, 4)), DMA((2, 2)), DMA((2, 2)), DMA((NB,)), DMA((4,)),
            ],
            compiler_params=pltpu.CompilerParams(vmem_limit_bytes=vmem*1024*1024, flags=flags, disable_bounds_checks=True),
            name="attn_v8",
        )(fx(A_x), t(A_k), t(A_v), A_wq, fo(A_wo), fx(B_x), t(B_k), t(B_v), B_wq, fo(B_wo))
        return out.reshape(B, Sq, 2*D)
    return f


_impl = build(lag=2, order='psf', rg=80, qw=128, ow=384, f0=1, so=(0,2,1), L_=dict(lag=1,order='fspf',ow=128,f0=0))


@jax.jit
def pallas_concat_heads__gqa_block_cached__mha_block_cached__near_ridge_kernel(
    A_x, A_k_cache, A_v_cache, A_wq, A_wo, B_x, B_k_cache, B_v_cache, B_wq, B_wo
):
    return _impl(A_x, A_k_cache, A_v_cache, A_wq, A_wo, B_x, B_k_cache, B_v_cache, B_wq, B_wo)
```

```python
import jax
import jax.numpy as jnp
import numpy as np
from jax import lax
import jax.experimental.pallas as pl
import jax.experimental.pallas.tpu as pltpu

B, SQ, D, H, SK, DH = 16, 160, 640, 32, 512, 192
G, BB = 4, 2
NG, NB = H // G, B // BB
M, W, HQ = BB * SQ, G * DH, SQ // 2
SPG = NB // 2
STEPS = NG * SPG
AHEAD = SPG + 1
SLOTS = 3
PSLOTS = 8
SCALE = float(DH**-0.5 * np.log2(np.e))
F32, BF16 = jnp.float32, jnp.bfloat16
NT = (((1,), (1,)), ((), ()))

MAIN_ORDER = "sqqsqpsqqpspsqqpsqqpsopsoopsoopsqqpsopsooopsoqpsqpsoopsooopsqpsqpsooopsoopsqpsqqpsoopsoopsoqpsqpsopsoooopsqpsqpsooopsoopqpqooooo"
TAIL_ORDER = "ssspspspspspspospospospospoospospospospoopopoooooooo"


def _kernel(ax, akt, avt, awq, awo, bx, bkt, bvt, bwq, bwo, out_hbm,
            xbuf, qbuf, kbuf, vbuf, wqbuf, wobuf, pbuf, acc, obuf,
            xsem, kvsem, wqsem, wosem, outsem, headsem):
    x_hbm, kv_hbm = (ax, bx), ((akt, avt), (bkt, bvt))
    wq_hbm, wo_hbm = (awq, bwq), (awo, bwo)
    copy = pltpu.make_async_copy

    def x_copy(src, r, k):
        rows = pl.ds(2 * k, 2)
        return copy(src.at[rows], xbuf.at[r, rows], xsem.at[r, k])

    def kv_copies(t, slot):
        return [copy(kv_hbm[r][e].at[t & (SPG - 1), :, t >> 2], buf.at[slot, r], kvsem.at[slot, r, e])
                for r in range(2) for e, buf in enumerate((kbuf, vbuf))]

    def wq_copy(r, g):
        cols = pl.ds(g * W if isinstance(g, int) else pl.multiple_of(g * W, 128), W)
        return copy(wq_hbm[r].at[:, cols], wqbuf.at[g & 1, r], wqsem.at[g & 1, r])

    def wo_copy(r, g):
        return copy(wo_hbm[r].at[g], wobuf.at[g & 1, r], wosem.at[g & 1, r])

    def out_copy(blk):
        return copy(obuf.at[blk], out_hbm.at[blk], outsem.at[blk])

    def start(copies):
        for c in copies:
            c.start()

    def wait(copies):
        for c in copies:
            c.wait()

    def rarely(cond, fn):
        lax.fori_loop(0, cond.astype(jnp.int32), lambda _, c: (fn(), c)[1], 0)

    low = lax.broadcasted_iota(jnp.int32, (HQ, 128), 1) < 64

    def sel(a, b):
        return jnp.where(low, a, b)

    def q_dot(r, blk, ws, c0, c1):
        return jnp.dot(xbuf[r, blk], wqbuf[ws, r, :, c0:c1], preferred_element_type=F32)

    def q_store(qslot, r, pair, q):
        q = q * SCALE
        for bb in range(BB):
            t, b = q[bb * SQ:bb * SQ + HQ], q[bb * SQ + HQ:(bb + 1) * SQ]
            t0, t1, t2 = t[:, :128], t[:, 128:256], t[:, 256:]
            b0, b1, b2 = b[:, :128], b[:, 128:256], b[:, 256:]
            c = sel(t1, b1)
            cr = pltpu.roll(c, 64, 1)
            even = [sel(t0 - b0, t0), sel(b1 - c, b0), sel(b0, cr)]
            odd = [sel(t2, t1 - c), sel(b2, b2 - t2), sel(cr, t2)]
            for e, parts in enumerate((even, odd)):
                qbuf[qslot + (r, bb, 2 * pair + e)] = jnp.concatenate(parts, axis=0).astype(BF16)

    def q_pair(qslot, r, blk, ws, pair):
        q_store(qslot, r, pair, q_dot(r, blk, ws, pair * 384, (pair + 1) * 384))

    def softmax(s):
        p = jnp.exp2(s - jnp.max(s, axis=-1, keepdims=True))
        l = jnp.sum(p, axis=-1, keepdims=True)
        inv = pl.reciprocal(l, approx=True)
        return p * (inv * (2.0 - l * inv))

    def region(order, t, halves, slot, qs, tail):
        g, blk0 = t >> 2, 2 * (t & (SPG - 1))
        wqs, qblk0 = ((t + AHEAD) >> 2) & 1, 2 * ((t + AHEAD) & (SPG - 1))
        units = [(h, r, bb, j) for h in range(len(halves)) for r in range(2)
                 for bb in range(BB) for j in range(G)]
        q_cols = [(h, r, c) for h in range(len(halves)) for r in range(2) for c in range(0, W, 128)]
        xyz, o_pairs, o_rows, q_parts, q_ready = {}, {}, {}, [], []

        def head_rows(ref, unit, a, b):
            h, r, bb, j = unit
            lead = (slot, r, halves[h] * BB + bb)
            rows = lambda k, n: ref[lead + (slice(j * DH + 64 * k, j * DH + 64 * k + n),)]
            return rows(a, 128) if b == a + 1 else jnp.concatenate([rows(a, 64), rows(b, 64)], axis=0)

        def scores(i):
            h, r, bb, j = units[i]
            blocks = [(0, 1), (2, 1), (0, 2)] if j % 2 == 0 else [(1, 0), (1, 2), (0, 2)]
            d = {e: jnp.dot(qbuf[qs, halves[h], r, bb, j, e * HQ:(e + 1) * HQ],
                            head_rows(kbuf, units[i], *blocks[e]), preferred_element_type=F32)
                 for e in (0, 2, 1)}
            p_t, p_b = softmax(d[0] + d[2]), softmax(d[1] + d[2])
            for e, p in enumerate((p_t, p_b, p_t - p_b)):
                for c in range(SK // 128):
                    pbuf[i % PSLOTS, e, c] = p[:, c * 128:(c + 1) * 128].astype(BF16)

        def values(i):
            odd = units[i][3] % 2
            blocks = [(1, 0), (2, 1), (2, 0)] if odd else [(0, 1), (1, 2), (0, 2)]
            xyz[i] = []
            for e in range(3):
                v = head_rows(vbuf, units[i], *blocks[e])
                d = [lax.dot_general(pbuf[i % PSLOTS, e, c], v[:, c * 128:(c + 1) * 128], NT,
                                     preferred_element_type=F32) for c in range(SK // 128)]
                xyz[i].append((d[0] + d[1]) + (d[2] + d[3]))
            if odd:
                (x0, y0, z0), (x1, y1, z1) = xyz[i - 1], xyz[i]
                o_pairs[i // 2] = jnp.concatenate([
                    jnp.concatenate([sel(x0, z0 + y0), sel(x0 - z0, y0)], axis=0),
                    jnp.concatenate([sel(x1, x0), pltpu.roll(sel(y0, y1), 64, 1)], axis=0),
                    jnp.concatenate([sel(z1 + y1, x1), sel(y1, x1 - z1)], axis=0)], axis=1)

        def out_proj(i):
            k, c = divmod(i, D // 128)
            h, r, bb, _ = units[k * G]
            if k not in o_rows:
                o_rows[k] = jnp.concatenate(
                    [o_pairs[k * G // 2 + n] for n in range(G // 2)], axis=1).astype(BF16)
            w = jnp.concatenate(
                [wobuf[g & 1, r, n * 384 + 64 * m:n * 384 + 64 * m + 64, c * 128:(c + 1) * 128]
                 for n in range(G // 2) for m in (0, 2, 4, 1, 5, 3)], axis=0)
            idx = (blk0 + halves[h], slice(bb * SQ, (bb + 1) * SQ),
                   slice(r * D + c * 128, r * D + (c + 1) * 128))
            prev = acc[idx]
            if not tail:
                prev = jnp.where(jnp.full(prev.shape, g, jnp.int32) > 0, prev, 0.0)
            res = prev + jnp.dot(o_rows[k], w, preferred_element_type=F32)
            acc[idx] = res
            if tail:
                obuf[idx] = res.astype(BF16)

        def q_proj(i):
            h, r, c = q_cols[i]
            q_parts.append(q_dot(r, qblk0 + h, wqs, c, c + 128))
            if len(q_parts) == 3:
                q_ready.append((h, r, c // 384, jnp.concatenate(q_parts, axis=1)))
                q_parts.clear()

        ops = dict(s=scores, p=values, o=out_proj, q=q_proj)
        count = dict(s=0, p=0, o=0, q=0)
        for op in order:
            ops[op](count[op])
            count[op] += 1
            assert 0 <= count["s"] - count["p"] <= PSLOTS
            while q_ready and units.index(q_ready[0][:2] + (BB - 1, 2 * q_ready[0][2] + 1)) < count["s"]:
                h, r, pair, q = q_ready.pop(0)
                q_store((qs, h), r, pair, q)
        n = len(units)
        assert count == dict(s=n, p=n, o=n // G * D // 128, q=0 if tail else len(q_cols))

    head = [copy(awq.at[:, 0:384], wqbuf.at[0, 0, :, 0:384], headsem.at[0]),
            copy(ax.at[0], xbuf.at[0, 0], headsem.at[1]),
            copy(awq.at[:, 384:W], wqbuf.at[0, 0, :, 384:W], headsem.at[2]),
            copy(ax.at[1], xbuf.at[0, 1], headsem.at[3])]
    start(head + [x_copy(ax, 0, k) for k in range(1, SPG)])
    wait(head[:2])
    q_pair((0, 0), 0, 0, 0, 0)
    start([wq_copy(1, 0)] + [x_copy(bx, 1, k) for k in range(SPG)] + [wq_copy(r, 1) for r in range(2)])
    wait(head[2:])
    q_pair((0, 0), 0, 0, 0, 1)
    q_pair((0, 1), 0, 1, 0, 0)
    q_pair((0, 1), 0, 1, 0, 1)
    start(kv_copies(0, 0) + [wo_copy(r, 0) for r in range(2)])

    def prologue(i, carry):
        late = i >= 2 * SPG
        r = jnp.where(late, i & 1, i >> 2)
        k = jnp.where(late, 0, i & (SPG - 1))
        ws = late.astype(jnp.int32)
        for rr in range(2):
            pl.when(i >> 2 == rr)(lambda: x_copy(x_hbm[rr], rr, k).wait())

        @pl.when(i == SPG)
        def _():
            wq_copy(1, 0).wait()
            start(kv_copies(1, 1))

        pl.when(i == 2 * SPG)(lambda: wait([wq_copy(rr, 1) for rr in range(2)]))
        for h in range(2):
            for pair in range(G // 2):
                q_pair((ws * SPG + k, h), r, 2 * k + h, ws, pair)
        return carry

    lax.fori_loop(1, 2 * AHEAD, prologue, 0)
    start([wq_copy(r, 2) for r in range(2)])

    def advance(i, n):
        return jnp.where(i == n - 1, 0, i + 1)

    def start_kv(t, slot):
        start(kv_copies(t + SLOTS - 1, jnp.where(slot == 0, SLOTS - 1, slot - 1)))

    def main_step(t, carry):
        slot, qs = carry
        start_kv(t, slot)
        new_wo, new_wq = (t & (SPG - 1)) == 0, ((t + AHEAD) & (SPG - 1)) == 0

        def weights():
            for new, weight_copy, g in ((new_wo, wo_copy, t >> 2), (new_wq, wq_copy, (t + AHEAD) >> 2)):
                pl.when(new)(lambda: wait([weight_copy(r, g) for r in range(2)]))
                pl.when(new & (g + 1 < NG))(lambda: start([weight_copy(r, g + 1) for r in range(2)]))

        rarely(new_wo | new_wq, weights)
        wait(kv_copies(t, slot))
        region(MAIN_ORDER, t, (0, 1), slot, qs, False)
        return advance(slot, SLOTS), advance(qs, AHEAD)

    def tail_step(n, carry):
        slot, qs = carry
        t, h = n >> 1, n & 1

        def loads():
            pl.when(t + SLOTS - 1 < STEPS)(lambda: start_kv(t, slot))
            pl.when(t == STEPS - SPG)(lambda: wait([wo_copy(r, NG - 1) for r in range(2)]))
            wait(kv_copies(t, slot))

        rarely(h == 0, loads)
        region(TAIL_ORDER, t, (h,), slot, qs, True)
        pl.when(t >= STEPS - SPG)(lambda: out_copy(n & (NB - 1)).start())
        return jnp.where(h == 1, advance(slot, SLOTS), slot), jnp.where(h == 1, advance(qs, AHEAD), qs)

    carry = lax.fori_loop(0, STEPS - AHEAD, main_step, (0, 0))
    lax.fori_loop(2 * (STEPS - AHEAD), 2 * STEPS, tail_step, carry)
    wait([out_copy(blk) for blk in range(NB)])


@jax.jit
def pallas_concat_heads__gqa_block_cached__mha_block_cached__near_ridge_kernel(
    A_x: jax.Array,
    A_k_cache: jax.Array,
    A_v_cache: jax.Array,
    A_wq: jax.Array,
    A_wo: jax.Array,
    B_x: jax.Array,
    B_k_cache: jax.Array,
    B_v_cache: jax.Array,
    B_wq: jax.Array,
    B_wo: jax.Array,
):
    def branch(x, k, v, wq, wo):
        assert x.shape == (B, SQ, D) and k.shape == v.shape == (B, H, SK, DH)
        cache = lambda a: jnp.swapaxes(a, 2, 3).reshape(SPG, 2 * BB, NG, W, SK)
        return x.reshape(NB, M, D), cache(k), cache(v), wq, wo.reshape(NG, W, D)

    dma = pltpu.SemaphoreType.DMA
    out = pl.pallas_call(
        _kernel,
        in_specs=[pl.BlockSpec(memory_space=pl.ANY)] * 10,
        out_specs=pl.BlockSpec(memory_space=pl.ANY),
        out_shape=jax.ShapeDtypeStruct((NB, M, 2 * D), BF16),
        scratch_shapes=[
            pltpu.VMEM((2, NB, M, D), BF16),
            pltpu.VMEM((AHEAD, 2, 2, BB, G, 3 * HQ, 128), BF16),
            pltpu.VMEM((SLOTS, 2, 2 * BB, W, SK), BF16),
            pltpu.VMEM((SLOTS, 2, 2 * BB, W, SK), BF16),
            pltpu.VMEM((2, 2, D, W), BF16),
            pltpu.VMEM((2, 2, W, D), BF16),
            pltpu.VMEM((PSLOTS, 3, SK // 128, HQ, 128), BF16),
            pltpu.VMEM((NB, M, 2 * D), F32),
            pltpu.VMEM((NB, M, 2 * D), BF16),
            dma((2, SPG)), dma((SLOTS, 2, 2)), dma((2, 2)), dma((2, 2)), dma((NB,)), dma((4,)),
        ],
        compiler_params=pltpu.CompilerParams(
            vmem_limit_bytes=120 * 1024 * 1024, disable_bounds_checks=True),
        name="attn_ab",
    )(*branch(A_x, A_k_cache, A_v_cache, A_wq, A_wo), *branch(B_x, B_k_cache, B_v_cache, B_wq, B_wo))
    return out.reshape(B, SQ, 2 * D)
```

```python
import jax
import jax.numpy as jnp
import numpy as np
from jax import lax
import jax.experimental.pallas as pl
import jax.experimental.pallas.tpu as pltpu

B, SQ, D, H, SK, DH = 16, 160, 640, 32, 512, 192
G, BB = 4, 2
NG, NB = H // G, B // BB
M, W, HQ = BB * SQ, G * DH, SQ // 2
SPG = NB // 2
STEPS = NG * SPG
AHEAD = SPG + 1
SLOTS = 3
PSLOTS = 8
SCALE = float(DH**-0.5 * np.log2(np.e))
F32, BF16 = jnp.float32, jnp.bfloat16
NT = (((1,), (1,)), ((), ()))

MAIN_ORDER = "sqsqqpsqqpspsqqpspqsqopsooopsposqqspopsooopsqqpspospspoopoosoqsqsoopsqospoqpoppsoqsopsoopsoqpsqpsopsoooopsqpsqpsooopsoopqpqooooo"
TAIL_ORDER = "ssspspspspspspospopsospoosposposopspospopoopoooooooo"


def _kernel(ax, akt, avt, awq, awo, bx, bkt, bvt, bwq, bwo, out_hbm,
            xbuf, qbuf, kbuf, vbuf, wqbuf, wobuf, pbuf, acc, obuf,
            xsem, kvsem, wqsem, wosem, outsem, headsem):
    x_hbm, kv_hbm = (ax, bx), ((akt, avt), (bkt, bvt))
    wq_hbm, wo_hbm = (awq, bwq), (awo, bwo)
    copy = pltpu.make_async_copy

    def x_copy(src, r, k):
        rows = pl.ds(2 * k, 2)
        return copy(src.at[rows], xbuf.at[r, rows], xsem.at[r, k])

    def kv_copies(t, slot):
        return [copy(kv_hbm[r][e].at[t & (SPG - 1), :, t >> 2], buf.at[slot, r], kvsem.at[slot, r, e])
                for r in range(2) for e, buf in enumerate((kbuf, vbuf))]

    def wq_copy(r, g):
        cols = pl.ds(g * W if isinstance(g, int) else pl.multiple_of(g * W, 128), W)
        return copy(wq_hbm[r].at[:, cols], wqbuf.at[g & 1, r], wqsem.at[g & 1, r])

    def wo_copy(r, g):
        return copy(wo_hbm[r].at[g], wobuf.at[g & 1, r], wosem.at[g & 1, r])

    def out_copy(blk):
        return copy(obuf.at[blk], out_hbm.at[blk], outsem.at[blk])

    def start(copies):
        for c in copies:
            c.start()

    def wait(copies):
        for c in copies:
            c.wait()

    def rarely(cond, fn):
        lax.fori_loop(0, cond.astype(jnp.int32), lambda _, c: (fn(), c)[1], 0)

    low = lax.broadcasted_iota(jnp.int32, (HQ, 128), 1) < 64

    def sel(a, b):
        return jnp.where(low, a, b)

    def q_dot(r, blk, ws, c0, c1):
        return jnp.dot(xbuf[r, blk], wqbuf[ws, r, :, c0:c1], preferred_element_type=F32)

    def q_store(qslot, r, pair, q):
        q = q * SCALE
        for bb in range(BB):
            t, b = q[bb * SQ:bb * SQ + HQ], q[bb * SQ + HQ:(bb + 1) * SQ]
            t0, t1, t2 = t[:, :128], t[:, 128:256], t[:, 256:]
            b0, b1, b2 = b[:, :128], b[:, 128:256], b[:, 256:]
            c = sel(t1, b1)
            cr = pltpu.roll(c, 64, 1)
            even = [sel(t0 - b0, t0), sel(b1 - c, b0), sel(b0, cr)]
            odd = [sel(t2, t1 - c), sel(b2, b2 - t2), sel(cr, t2)]
            for e, parts in enumerate((even, odd)):
                qbuf[qslot + (r, bb, 2 * pair + e)] = jnp.concatenate(parts, axis=0).astype(BF16)

    def q_pair(qslot, r, blk, ws, pair):
        q_store(qslot, r, pair, q_dot(r, blk, ws, pair * 384, (pair + 1) * 384))

    def softmax(s):
        p = jnp.exp2(s - jnp.max(s, axis=-1, keepdims=True))
        l = jnp.sum(p, axis=-1, keepdims=True)
        inv = pl.reciprocal(l, approx=True)
        return p * (inv * (2.0 - l * inv))

    def region(order, t, halves, slot, qs, tail):
        g, blk0 = t >> 2, 2 * (t & (SPG - 1))
        wqs, qblk0 = ((t + AHEAD) >> 2) & 1, 2 * ((t + AHEAD) & (SPG - 1))
        units = [(h, r, bb, j) for h in range(len(halves)) for r in range(2)
                 for bb in range(BB) for j in range(G)]
        q_cols = [(h, r, c) for h in range(len(halves)) for r in range(2) for c in range(0, W, 128)]
        xyz, o_pairs, o_rows, q_parts, q_ready = {}, {}, {}, [], []

        def head_rows(ref, unit, e, a, b):
            h, r, bb, j = unit
            lead = (slot[e], r, halves[h] * BB + bb)
            rows = lambda k, n: ref[lead + (slice(j * DH + 64 * k, j * DH + 64 * k + n),)]
            return rows(a, 128) if b == a + 1 else jnp.concatenate([rows(a, 64), rows(b, 64)], axis=0)

        def scores(i):
            h, r, bb, j = units[i]
            blocks = [(0, 1), (2, 1), (0, 2)] if j % 2 == 0 else [(1, 0), (1, 2), (0, 2)]
            d = {e: jnp.dot(qbuf[qs, halves[h], r, bb, j, e * HQ:(e + 1) * HQ],
                            head_rows(kbuf, units[i], e, *blocks[e]), preferred_element_type=F32)
                 for e in (2, 0, 1)}
            p_t, p_b = softmax(d[2] + d[0]), softmax(d[2] + d[1])
            for e, p in enumerate((p_t, p_b, p_t - p_b)):
                for c in range(SK // 128):
                    pbuf[i % PSLOTS, e, c] = p[:, c * 128:(c + 1) * 128].astype(BF16)

        def values(i):
            odd = units[i][3] % 2
            blocks = [(1, 0), (2, 1), (2, 0)] if odd else [(0, 1), (1, 2), (0, 2)]
            xyz[i] = []
            for e in range(3):
                v = head_rows(vbuf, units[i], e, *blocks[e])
                d = [lax.dot_general(pbuf[i % PSLOTS, e, c], v[:, c * 128:(c + 1) * 128], NT,
                                     preferred_element_type=F32) for c in range(SK // 128)]
                xyz[i].append((d[0] + d[1]) + (d[2] + d[3]))
            if odd:
                (x0, y0, z0), (x1, y1, z1) = xyz[i - 1], xyz[i]
                o_pairs[i // 2] = jnp.concatenate([
                    jnp.concatenate([sel(x0, z0 + y0), sel(x0 - z0, y0)], axis=0),
                    jnp.concatenate([sel(x1, x0), pltpu.roll(sel(y0, y1), 64, 1)], axis=0),
                    jnp.concatenate([sel(z1 + y1, x1), sel(y1, x1 - z1)], axis=0)], axis=1)

        def out_proj(i):
            k, c = divmod(i, D // 128)
            h, r, bb, _ = units[k * G]
            if k not in o_rows:
                o_rows[k] = jnp.concatenate(
                    [o_pairs[k * G // 2 + n] for n in range(G // 2)], axis=1).astype(BF16)
            w = jnp.concatenate(
                [wobuf[g & 1, r, n * 384 + 64 * m:n * 384 + 64 * m + 64, c * 128:(c + 1) * 128]
                 for n in range(G // 2) for m in (0, 2, 4, 1, 5, 3)], axis=0)
            idx = (blk0 + halves[h], slice(bb * SQ, (bb + 1) * SQ),
                   slice(r * D + c * 128, r * D + (c + 1) * 128))
            prev = acc[idx]
            if not tail:
                prev = jnp.where(jnp.full(prev.shape, g, jnp.int32) > 0, prev, 0.0)
            res = prev + jnp.dot(o_rows[k], w, preferred_element_type=F32)
            acc[idx] = res
            if tail:
                obuf[idx] = res.astype(BF16)

        def q_proj(i):
            h, r, c = q_cols[i]
            q_parts.append(q_dot(r, qblk0 + h, wqs, c, c + 128))
            if len(q_parts) == 3:
                q_ready.append((h, r, c // 384, jnp.concatenate(q_parts, axis=1)))
                q_parts.clear()

        ops = dict(s=scores, p=values, o=out_proj, q=q_proj)
        count = dict(s=0, p=0, o=0, q=0)
        for op in order:
            ops[op](count[op])
            count[op] += 1
            assert 0 <= count["s"] - count["p"] <= PSLOTS
            while q_ready and units.index(q_ready[0][:2] + (BB - 1, 2 * q_ready[0][2] + 1)) < count["s"]:
                h, r, pair, q = q_ready.pop(0)
                q_store((qs, h), r, pair, q)
        n = len(units)
        assert count == dict(s=n, p=n, o=n // G * D // 128, q=0 if tail else len(q_cols))

    head = [copy(awq.at[:, 0:384], wqbuf.at[0, 0, :, 0:384], headsem.at[0]),
            copy(ax.at[0], xbuf.at[0, 0], headsem.at[1]),
            copy(awq.at[:, 384:W], wqbuf.at[0, 0, :, 384:W], headsem.at[2]),
            copy(ax.at[1], xbuf.at[0, 1], headsem.at[3])]
    start(head + [x_copy(ax, 0, k) for k in range(1, SPG)])
    wait(head[:2])
    q_pair((0, 0), 0, 0, 0, 0)
    start([wq_copy(1, 0)] + [x_copy(bx, 1, k) for k in range(SPG)] + [wq_copy(r, 1) for r in range(2)])
    wait(head[2:])
    q_pair((0, 0), 0, 0, 0, 1)
    q_pair((0, 1), 0, 1, 0, 0)
    q_pair((0, 1), 0, 1, 0, 1)
    start(kv_copies(0, 0) + [wo_copy(r, 0) for r in range(2)])

    def prologue(i, carry):
        late = i >= 2 * SPG
        r = jnp.where(late, i & 1, i >> 2)
        k = jnp.where(late, 0, i & (SPG - 1))
        ws = late.astype(jnp.int32)
        for rr in range(2):
            pl.when(i >> 2 == rr)(lambda: x_copy(x_hbm[rr], rr, k).wait())

        @pl.when(i == SPG)
        def _():
            wq_copy(1, 0).wait()
            start(kv_copies(1, 1))

        pl.when(i == 2 * SPG)(lambda: wait([wq_copy(rr, 1) for rr in range(2)]))
        for h in range(2):
            for pair in range(G // 2):
                q_pair((ws * SPG + k, h), r, 2 * k + h, ws, pair)
        return carry

    lax.fori_loop(1, 2 * AHEAD, prologue, 0)
    start([wq_copy(r, 2) for r in range(2)])

    def advance(i, n):
        return jnp.where(i == n - 1, 0, i + 1)

    def start_kv(t, slot):
        start(kv_copies(t + SLOTS - 1, jnp.where(slot == 0, SLOTS - 1, slot - 1)))

    def main_step(t, carry):
        slot, qs = carry
        start_kv(t, slot)
        new_wo, new_wq = (t & (SPG - 1)) == 0, ((t + AHEAD) & (SPG - 1)) == 0

        def weights():
            for new, weight_copy, g in ((new_wo, wo_copy, t >> 2), (new_wq, wq_copy, (t + AHEAD) >> 2)):
                pl.when(new)(lambda: wait([weight_copy(r, g) for r in range(2)]))
                pl.when(new & (g + 1 < NG))(lambda: start([weight_copy(r, g + 1) for r in range(2)]))

        rarely(new_wo | new_wq, weights)
        wait(kv_copies(t, slot))
        region(MAIN_ORDER, t, (0, 1), (slot, slot & 3, slot & 7), qs, False)
        return advance(slot, SLOTS), advance(qs, AHEAD)

    def tail_step(n, carry):
        slot, qs = carry
        t, h = n >> 1, n & 1

        def loads():
            pl.when(t + SLOTS - 1 < STEPS)(lambda: start_kv(t, slot))
            pl.when(t == STEPS - SPG)(lambda: wait([wo_copy(r, NG - 1) for r in range(2)]))
            wait(kv_copies(t, slot))

        rarely(h == 0, loads)
        region(TAIL_ORDER, t, (h,), (slot, slot & 3, slot & 7), qs, True)
        pl.when(t >= STEPS - SPG)(lambda: out_copy(n & (NB - 1)).start())
        return jnp.where(h == 1, advance(slot, SLOTS), slot), jnp.where(h == 1, advance(qs, AHEAD), qs)

    carry = lax.fori_loop(0, STEPS - AHEAD, main_step, (0, 0))
    lax.fori_loop(2 * (STEPS - AHEAD), 2 * STEPS, tail_step, carry)
    wait([out_copy(blk) for blk in range(NB)])


@jax.jit
def pallas_concat_heads__gqa_block_cached__mha_block_cached__near_ridge_kernel(
    A_x: jax.Array,
    A_k_cache: jax.Array,
    A_v_cache: jax.Array,
    A_wq: jax.Array,
    A_wo: jax.Array,
    B_x: jax.Array,
    B_k_cache: jax.Array,
    B_v_cache: jax.Array,
    B_wq: jax.Array,
    B_wo: jax.Array,
):
    def branch(x, k, v, wq, wo):
        assert x.shape == (B, SQ, D) and k.shape == v.shape == (B, H, SK, DH)
        cache = lambda a: jnp.swapaxes(a, 2, 3).reshape(SPG, 2 * BB, NG, W, SK)
        return x.reshape(NB, M, D), cache(k), cache(v), wq, wo.reshape(NG, W, D)

    dma = pltpu.SemaphoreType.DMA
    out = pl.pallas_call(
        _kernel,
        in_specs=[pl.BlockSpec(memory_space=pl.ANY)] * 10,
        out_specs=pl.BlockSpec(memory_space=pl.ANY),
        out_shape=jax.ShapeDtypeStruct((NB, M, 2 * D), BF16),
        scratch_shapes=[
            pltpu.VMEM((2, NB, M, D), BF16),
            pltpu.VMEM((AHEAD, 2, 2, BB, G, 3 * HQ, 128), BF16),
            pltpu.VMEM((SLOTS, 2, 2 * BB, W, SK), BF16),
            pltpu.VMEM((SLOTS, 2, 2 * BB, W, SK), BF16),
            pltpu.VMEM((2, 2, D, W), BF16),
            pltpu.VMEM((2, 2, W, D), BF16),
            pltpu.VMEM((PSLOTS, 3, SK // 128, HQ, 128), BF16),
            pltpu.VMEM((NB, M, 2 * D), F32),
            pltpu.VMEM((NB, M, 2 * D), BF16),
            dma((2, SPG)), dma((SLOTS, 2, 2)), dma((2, 2)), dma((2, 2)), dma((NB,)), dma((4,)),
        ],
        compiler_params=pltpu.CompilerParams(
            vmem_limit_bytes=120 * 1024 * 1024, disable_bounds_checks=True),
        name="attn_ab",
    )(*branch(A_x, A_k_cache, A_v_cache, A_wq, A_wo), *branch(B_x, B_k_cache, B_v_cache, B_wq, B_wo))
    return out.reshape(B, SQ, 2 * D)
```

```python
import jax
import jax.numpy as jnp
import numpy as np
from jax import lax
import jax.experimental.pallas as pl
import jax.experimental.pallas.tpu as pltpu

B, SQ, D, H, SK, DH = 16, 160, 640, 32, 512, 192
G, BB = 4, 2
NG, NB = H // G, B // BB
M, W, HQ = BB * SQ, G * DH, SQ // 2
SPG = NB // 2
STEPS = NG * SPG
AHEAD = SPG + 1
SLOTS = 3
PSLOTS = 8
SCALE = float(DH**-0.5 * np.log2(np.e))
F32, BF16 = jnp.float32, jnp.bfloat16
NT = (((1,), (1,)), ((), ()))

MAIN_ORDER = (
    "sqsqqpsqqpspsqqpspqsqopsooopsposqqspopsooopsqqpspospspoopoosoqsqsoopsqospoqpoppsoqsopsoopsoqpsqpsoopsooopspqsqpsoopsoopoqpqooooo"
)
TAIL_ORDER = "ssspspspspspspospopsospoosposposopspospopoopoooooooo"


def _kernel(ax, akt, avt, awq, awo, bx, bkt, bvt, bwq, bwo, out_hbm,
            xbuf, qbuf, kbuf, vbuf, wqbuf, wobuf, pbuf, acc, obuf,
            xsem, kvsem, wqsem, wosem, outsem, headsem):
    x_hbm, kv_hbm = (ax, bx), ((akt, avt), (bkt, bvt))
    wq_hbm, wo_hbm = (awq, bwq), (awo, bwo)
    copy = pltpu.make_async_copy

    def x_copy(src, r, k):
        rows = pl.ds(2 * k, 2)
        return copy(src.at[rows], xbuf.at[r, rows], xsem.at[r, k])

    def kv_copies(t, slot):
        return [copy(kv_hbm[r][e].at[t & (SPG - 1), :, t >> 2], buf.at[slot, r], kvsem.at[slot, r, e])
                for r in range(2) for e, buf in enumerate((kbuf, vbuf))]

    def wq_copy(r, g):
        cols = pl.ds(g * W if isinstance(g, int) else pl.multiple_of(g * W, 128), W)
        return copy(wq_hbm[r].at[:, cols], wqbuf.at[g & 1, r], wqsem.at[g & 1, r])

    def wo_copy(r, g):
        return copy(wo_hbm[r].at[g], wobuf.at[g & 1, r], wosem.at[g & 1, r])

    def out_copy(blk):
        return copy(obuf.at[blk], out_hbm.at[blk], outsem.at[blk])

    def start(copies):
        for c in copies:
            c.start()

    def wait(copies):
        for c in copies:
            c.wait()

    def rarely(cond, fn):
        lax.fori_loop(0, cond.astype(jnp.int32), lambda _, c: (fn(), c)[1], 0)

    low = lax.broadcasted_iota(jnp.int32, (HQ, 128), 1) < 64

    def sel(a, b):
        return jnp.where(low, a, b)

    def q_dot(r, blk, ws, c0, c1):
        return jnp.dot(xbuf[r, blk], wqbuf[ws, r, :, c0:c1], preferred_element_type=F32)

    def q_store(qslot, r, pair, q):
        q = q * SCALE
        for bb in range(BB):
            t, b = q[bb * SQ:bb * SQ + HQ], q[bb * SQ + HQ:(bb + 1) * SQ]
            t0, t1, t2 = t[:, :128], t[:, 128:256], t[:, 256:]
            b0, b1, b2 = b[:, :128], b[:, 128:256], b[:, 256:]
            c = sel(t1, b1)
            cr = pltpu.roll(c, 64, 1)
            even = [sel(t0 - b0, t0), sel(b1 - c, b0), sel(b0, cr)]
            odd = [sel(t2, t1 - c), sel(b2, b2 - t2), sel(cr, t2)]
            for e, parts in enumerate((even, odd)):
                qbuf[qslot + (r, bb, 2 * pair + e)] = jnp.concatenate(parts, axis=0).astype(BF16)

    def q_pair(qslot, r, blk, ws, pair):
        q_store(qslot, r, pair, q_dot(r, blk, ws, pair * 384, (pair + 1) * 384))

    def softmax(s):
        p = jnp.exp2(s - jnp.max(s, axis=-1, keepdims=True))
        l = jnp.sum(p, axis=-1, keepdims=True)
        inv = pl.reciprocal(l, approx=True)
        return p * (inv * (2.0 - l * inv))

    def region(order, t, halves, slot, qs, tail):
        g, blk0 = t >> 2, 2 * (t & (SPG - 1))
        wqs, qblk0 = ((t + AHEAD) >> 2) & 1, 2 * ((t + AHEAD) & (SPG - 1))
        units = [(h, r, bb, j) for h in range(len(halves)) for r in range(2)
                 for bb in range(BB) for j in range(G)]
        q_cols = [(h, r, c) for h in range(len(halves)) for r in range(2) for c in range(0, W, 128)]
        xyz, o_pairs, o_rows, q_parts, q_ready = {}, {}, {}, [], []

        slots = (slot, slot & 3, slot & 7)

        def head_rows(ref, unit, e, a, b):
            h, r, bb, j = unit
            lead = (slots[e], r, halves[h] * BB + bb)
            rows = lambda k, n: ref[lead + (slice(j * DH + 64 * k, j * DH + 64 * k + n),)]
            return rows(a, 128) if b == a + 1 else jnp.concatenate([rows(a, 64), rows(b, 64)], axis=0)

        def scores(i):
            h, r, bb, j = units[i]
            blocks = [(0, 1), (2, 1), (0, 2)] if j % 2 == 0 else [(1, 0), (1, 2), (0, 2)]
            d = {e: jnp.dot(qbuf[qs, halves[h], r, bb, j, e * HQ:(e + 1) * HQ],
                            head_rows(kbuf, units[i], e, *blocks[e]), preferred_element_type=F32)
                 for e in (2, 0, 1)}
            p_t, p_b = softmax(d[2] + d[0]), softmax(d[2] + d[1])
            for e, p in enumerate((p_t, p_b, p_t - p_b)):
                for c in range(SK // 128):
                    pbuf[i % PSLOTS, e, c] = p[:, c * 128:(c + 1) * 128].astype(BF16)

        def values(i):
            odd = units[i][3] % 2
            blocks = [(1, 0), (2, 1), (2, 0)] if odd else [(0, 1), (1, 2), (0, 2)]
            xyz[i] = []
            for e in range(3):
                v = head_rows(vbuf, units[i], e, *blocks[e])
                d = [lax.dot_general(pbuf[i % PSLOTS, e, c], v[:, c * 128:(c + 1) * 128], NT,
                                     preferred_element_type=F32) for c in range(SK // 128)]
                xyz[i].append((d[0] + d[1]) + (d[2] + d[3]))
            if odd:
                (x0, y0, z0), (x1, y1, z1) = xyz[i - 1], xyz[i]
                o_pairs[i // 2] = jnp.concatenate([
                    jnp.concatenate([sel(x0, z0 + y0), sel(x0 - z0, y0)], axis=0),
                    jnp.concatenate([sel(x1, x0), pltpu.roll(sel(y0, y1), 64, 1)], axis=0),
                    jnp.concatenate([sel(z1 + y1, x1), sel(y1, x1 - z1)], axis=0)], axis=1)

        def out_proj(i):
            k, c = divmod(i, D // 128)
            h, r, bb, _ = units[k * G]
            if k not in o_rows:
                o_rows[k] = jnp.concatenate(
                    [o_pairs[k * G // 2 + n] for n in range(G // 2)], axis=1).astype(BF16)
            w = jnp.concatenate(
                [wobuf[g & 1, r, n * 384 + 64 * m:n * 384 + 64 * m + 64, c * 128:(c + 1) * 128]
                 for n in range(G // 2) for m in (0, 2, 4, 1, 5, 3)], axis=0)
            idx = (blk0 + halves[h], slice(bb * SQ, (bb + 1) * SQ),
                   slice(r * D + c * 128, r * D + (c + 1) * 128))
            prev = acc[idx]
            if not tail:
                prev = jnp.where(jnp.full(prev.shape, g, jnp.int32) > 0, prev, 0.0)
            res = prev + jnp.dot(o_rows[k], w, preferred_element_type=F32)
            acc[idx] = res
            if tail:
                obuf[idx] = res.astype(BF16)

        def q_proj(i):
            h, r, c = q_cols[i]
            q_parts.append(q_dot(r, qblk0 + h, wqs, c, c + 128))
            if len(q_parts) == 3:
                q_ready.append((h, r, c // 384, jnp.concatenate(q_parts, axis=1)))
                q_parts.clear()

        ops = dict(s=scores, p=values, o=out_proj, q=q_proj)
        count = dict(s=0, p=0, o=0, q=0)
        for op in order:
            ops[op](count[op])
            count[op] += 1
            assert 0 <= count["s"] - count["p"] <= PSLOTS
            while q_ready and units.index(q_ready[0][:2] + (BB - 1, 2 * q_ready[0][2] + 1)) < count["s"]:
                h, r, pair, q = q_ready.pop(0)
                q_store((qs, h), r, pair, q)
        n = len(units)
        assert count == dict(s=n, p=n, o=n // G * D // 128, q=0 if tail else len(q_cols))

    head = [copy(awq.at[:, 0:384], wqbuf.at[0, 0, :, 0:384], headsem.at[0]),
            copy(ax.at[0], xbuf.at[0, 0], headsem.at[1]),
            copy(awq.at[:, 384:W], wqbuf.at[0, 0, :, 384:W], headsem.at[2]),
            copy(ax.at[1], xbuf.at[0, 1], headsem.at[3])]
    start(head + [x_copy(ax, 0, k) for k in range(1, SPG)])
    wait(head[:2])
    q_pair((0, 0), 0, 0, 0, 0)
    start([wq_copy(1, 0)] + [x_copy(bx, 1, k) for k in range(SPG)] + [wq_copy(r, 1) for r in range(2)])
    wait(head[2:])
    q_pair((0, 0), 0, 0, 0, 1)
    q_pair((0, 1), 0, 1, 0, 0)
    q_pair((0, 1), 0, 1, 0, 1)
    start(kv_copies(0, 0) + [wo_copy(r, 0) for r in range(2)])

    def prologue(i, carry):
        late = i >= 2 * SPG
        r = jnp.where(late, i & 1, i >> 2)
        k = jnp.where(late, 0, i & (SPG - 1))
        ws = late.astype(jnp.int32)
        for rr in range(2):
            pl.when(i >> 2 == rr)(lambda: x_copy(x_hbm[rr], rr, k).wait())

        @pl.when(i == SPG)
        def _():
            wq_copy(1, 0).wait()
            start(kv_copies(1, 1))

        pl.when(i == 2 * SPG)(lambda: wait([wq_copy(rr, 1) for rr in range(2)]))
        for h in range(2):
            for pair in range(G // 2):
                q_pair((ws * SPG + k, h), r, 2 * k + h, ws, pair)
        return carry

    lax.fori_loop(1, 2 * AHEAD, prologue, 0)
    start([wq_copy(r, 2) for r in range(2)])

    def advance(i, n):
        return jnp.where(i == n - 1, 0, i + 1)

    def start_kv(t, slot):
        start(kv_copies(t + SLOTS - 1, jnp.where(slot == 0, SLOTS - 1, slot - 1)))

    def main_step(t, carry):
        slot, qs = carry
        start_kv(t, slot)
        new_wo, new_wq = (t & (SPG - 1)) == 0, ((t + AHEAD) & (SPG - 1)) == 0

        def weights():
            for new, weight_copy, g in ((new_wo, wo_copy, t >> 2), (new_wq, wq_copy, (t + AHEAD) >> 2)):
                pl.when(new)(lambda: wait([weight_copy(r, g) for r in range(2)]))
                pl.when(new & (g + 1 < NG))(lambda: start([weight_copy(r, g + 1) for r in range(2)]))

        rarely(new_wo | new_wq, weights)
        wait(kv_copies(t, slot))
        region(MAIN_ORDER, t, (0, 1), slot, qs, False)
        return advance(slot, SLOTS), advance(qs, AHEAD)

    def tail_step(n, carry):
        slot, qs = carry
        t, h = n >> 1, n & 1

        def loads():
            pl.when(t + SLOTS - 1 < STEPS)(lambda: start_kv(t, slot))
            pl.when(t == STEPS - SPG)(lambda: wait([wo_copy(r, NG - 1) for r in range(2)]))
            wait(kv_copies(t, slot))

        rarely(h == 0, loads)
        region(TAIL_ORDER, t, (h,), slot, qs, True)
        pl.when(t >= STEPS - SPG)(lambda: out_copy(n & (NB - 1)).start())
        return jnp.where(h == 1, advance(slot, SLOTS), slot), jnp.where(h == 1, advance(qs, AHEAD), qs)

    carry = lax.fori_loop(0, STEPS - AHEAD, main_step, (0, 0))
    lax.fori_loop(2 * (STEPS - AHEAD), 2 * STEPS, tail_step, carry)
    wait([out_copy(blk) for blk in range(NB)])


@jax.jit
def pallas_concat_heads__gqa_block_cached__mha_block_cached__near_ridge_kernel(
    A_x: jax.Array,
    A_k_cache: jax.Array,
    A_v_cache: jax.Array,
    A_wq: jax.Array,
    A_wo: jax.Array,
    B_x: jax.Array,
    B_k_cache: jax.Array,
    B_v_cache: jax.Array,
    B_wq: jax.Array,
    B_wo: jax.Array,
):
    def branch(x, k, v, wq, wo):
        assert x.shape == (B, SQ, D) and k.shape == v.shape == (B, H, SK, DH)
        cache = lambda a: jnp.swapaxes(a, 2, 3).reshape(SPG, 2 * BB, NG, W, SK)
        return x.reshape(NB, M, D), cache(k), cache(v), wq, wo.reshape(NG, W, D)

    dma = pltpu.SemaphoreType.DMA
    out = pl.pallas_call(
        _kernel,
        in_specs=[pl.BlockSpec(memory_space=pl.ANY)] * 10,
        out_specs=pl.BlockSpec(memory_space=pl.ANY),
        out_shape=jax.ShapeDtypeStruct((NB, M, 2 * D), BF16),
        scratch_shapes=[
            pltpu.VMEM((2, NB, M, D), BF16),
            pltpu.VMEM((AHEAD, 2, 2, BB, G, 3 * HQ, 128), BF16),
            pltpu.VMEM((SLOTS, 2, 2 * BB, W, SK), BF16),
            pltpu.VMEM((SLOTS, 2, 2 * BB, W, SK), BF16),
            pltpu.VMEM((2, 2, D, W), BF16),
            pltpu.VMEM((2, 2, W, D), BF16),
            pltpu.VMEM((PSLOTS, 3, SK // 128, HQ, 128), BF16),
            pltpu.VMEM((NB, M, 2 * D), F32),
            pltpu.VMEM((NB, M, 2 * D), BF16),
            dma((2, SPG)), dma((SLOTS, 2, 2)), dma((2, 2)), dma((2, 2)), dma((NB,)), dma((4,)),
        ],
        compiler_params=pltpu.CompilerParams(
            vmem_limit_bytes=100 * 1024 * 1024, disable_bounds_checks=True),
        name="attn_ab",
    )(*branch(A_x, A_k_cache, A_v_cache, A_wq, A_wo), *branch(B_x, B_k_cache, B_v_cache, B_wq, B_wo))
    return out.reshape(B, SQ, 2 * D)
```
